```python
import jax
import jax.numpy as jnp

def _softmax(x, axis=-1):
    return jax.nn.softmax(x, axis=axis)
def _gelu(x):
    return jax.nn.gelu(x, approximate=True)
def _silu(x):
    return jax.nn.silu(x)
def _sigmoid(x):
    return jax.nn.sigmoid(x)
def _layernorm(x, axis=-1, eps=1e-5):
    m = jnp.mean(x, axis=axis, keepdims=True)
    v = jnp.var(x, axis=axis, keepdims=True)
    return (x - m) / jnp.sqrt(v + eps)
def _scatter_add(tgt, idx, src, axis=0):
    return tgt.at[idx].add(src)
def _segment_sum(src, seg, n):
    return jax.ops.segment_sum(src, seg, n)
class _Rng:
    def __init__(self, key):
        self._k = key
    def _next(self):
        self._k, sub = jax.random.split(self._k)
        return sub
    def normal(self, shape):
        return jax.random.normal(self._next(), shape, dtype=jnp.bfloat16)
    def randint(self, lo, hi, shape):
        return jax.random.randint(self._next(), shape, lo, hi, dtype=jnp.int32)
    def uniform(self, shape, lo=0.0, hi=1.0):
        return jax.random.uniform(self._next(), shape, jnp.bfloat16, lo, hi)
    def permutation(self, n):
        return jax.random.permutation(self._next(), n)


kernel_name = 'parallel_sum__compressed_kv_cla__moe_arch_mod__prompt'

def setup_inputs():
    _rng = _Rng(jax.random.key(int.from_bytes(__import__("os").urandom(4), "little")))
    _w = (lambda a: (lambda t: t.astype(jnp.bfloat16) if jnp.issubdtype(t.dtype, jnp.floating) else t)(jnp.asarray(a)))
    def _A_setup():
        B, H, Sq, Sk, D, M = 1, 32, 2048, 2048, 128, 640
        Dc = 4 * D
        return {
            "x": _w((lambda *s: _rng.normal(s) * 0.05)(B, Sq, M)),
            "c_kv": _w((lambda *s: _rng.normal(s) * 0.05)(B, Sk, Dc)),
            "w_q": _w((lambda *s: _rng.normal(s) * 0.05)(M, H, D) * (M ** -0.5)),
            "w_uk": _w((lambda *s: _rng.normal(s) * 0.05)(Dc, H, D) * (Dc ** -0.5)),
            "w_uv": _w((lambda *s: _rng.normal(s) * 0.05)(Dc, H, D) * (Dc ** -0.5)),
            "w_o": _w((lambda *s: _rng.normal(s) * 0.05)(H, D, M) * ((H * D) ** -0.5)),
        }
    _A_in = _A_setup()

    def _B_setup():
        B, S, D, F, C = 1, 2048, 640, 1728, 8
        return {
            "x": _w((lambda *s: _rng.normal(s) * 0.05)(B, S, D)),
            "w_r": _w((lambda *s: _rng.normal(s) * 0.05)(D)),
            "w_gate": _w((lambda *s: _rng.normal(s) * 0.05)(D, F)),
            "w_up": _w((lambda *s: _rng.normal(s) * 0.05)(D, F)),
            "w_down": _w((lambda *s: _rng.normal(s) * 0.05)(F, D)),
        }
    _B_in = _B_setup()

    return {
        "A_x": _A_in["x"],
        "A_c_kv": _A_in["c_kv"],
        "A_w_q": _A_in["w_q"],
        "A_w_uk": _A_in["w_uk"],
        "A_w_uv": _A_in["w_uv"],
        "A_w_o": _A_in["w_o"],
        "B_x": _B_in["x"],
        "B_w_r": _B_in["w_r"],
        "B_w_gate": _B_in["w_gate"],
        "B_w_up": _B_in["w_up"],
        "B_w_down": _B_in["w_down"],
    }

def reference(A_x, A_c_kv, A_w_q, A_w_uk, A_w_uv, A_w_o, B_x, B_w_r, B_w_gate, B_w_up, B_w_down):
    def _A_ref(x, c_kv, w_q, w_uk, w_uv, w_o):
        B, Sq, M = x.shape[0], x.shape[1], x.shape[2]
        Sk = c_kv.shape[1]
        H, D = w_q.shape[1], w_q.shape[2]
        q = jnp.einsum("bqm,mhd->bhqd", x, w_q)
        k = jnp.einsum("bkc,chd->bhkd", c_kv, w_uk)
        v = jnp.einsum("bkc,chd->bhkd", c_kv, w_uv)
        scores = jnp.einsum("bhqd,bhkd->bhqk", q, k) * (D ** -0.5)
        off = Sk - Sq
        qi = jnp.arange(Sq)[:, None]
        kj = jnp.arange(Sk)[None, :]
        cmask = kj <= (qi + off)
        scores = jnp.where(cmask[None, None], scores, -1e9)
        p = _softmax(scores, axis=-1)
        ctx = jnp.einsum("bhqk,bhkd->bhqd", p, v)
        return jnp.einsum("bhqd,hdm->bqm", ctx, w_o)

    def _B_ref(x, w_r, w_gate, w_up, w_down):
        B, S, D = x.shape
        C = 8
        r = x @ w_r
        idx = jnp.argsort(-r, axis=-1)[:, :C]
        idx_e = jnp.repeat(idx.reshape(B, C, 1), D, axis=2)
        x_sel = jnp.take_along_axis(x, idx_e, axis=1)
        g = _silu(x_sel @ w_gate)
        u = x_sel @ w_up
        y = (g * u) @ w_down
        r_sel = _sigmoid(jnp.take_along_axis(r, idx, axis=1))
        y = y * r_sel.reshape(B, C, 1)
        b_off = (jnp.arange(B) * S).reshape(B, 1)
        flat_idx = (idx + b_off).reshape(B * C)
        zero = (x * 0.0).reshape(B * S, D)
        upd = _scatter_add(zero, flat_idx, y.reshape(B * C, D), axis=0)
        return x + upd.reshape(B, S, D)

    x = A_x
    xn = _layernorm(x, axis=-1)
    return x + _A_ref(xn, A_c_kv, A_w_q, A_w_uk, A_w_uv, A_w_o) + _B_ref(xn, B_w_r, B_w_gate, B_w_up, B_w_down)
```

```python
import math

import jax
import jax.numpy as jnp
import numpy as np
from jax import lax
from jax.experimental import pallas as pl
from jax.experimental.pallas import tpu as pltpu

F32, BF16, U32, I32 = jnp.float32, jnp.bfloat16, jnp.uint32, jnp.int32
L = 128
BQ = 512
TOPC = 8
NT = (((1,), (1,)), ((), ()))
LOG2E = math.log2(math.e)


def _round_bf16(x):
    return x.astype(BF16).astype(F32)


def _dot(a, b):
    return jnp.dot(a, b, preferred_element_type=F32)


def _dot_nt(a, b):
    return lax.dot_general(a, b, NT, preferred_element_type=F32)


def _half(u, hi):
    bits = (u & np.uint32(0xFFFF0000)) if hi else (u << 16)
    return pltpu.bitcast(bits, F32).astype(BF16)


def _kernel(x_hbm, c_hbm, wq_hbm, wk_hbm, wv_hbm, wo_hbm, wr_ref, wg_hbm, wu_hbm, wd_hbm,
            out_hbm,
            x_v, c_v, xn_v, acc_v, wq_v, wk_v, wv_v, wo_v, wg_v, wu_v, wd_v,
            qa, ka, va, qb, kb, vb, ctx_v, xs_v, gate_v, idx_s, sems, wsem, osem):
    S, M = x_v.shape
    n_pair = wq_hbm.shape[1] // 2
    nm, nc = xn_v.shape[0], c_v.shape[0]
    nq = S // BQ
    q_scale = float(np.float32(L ** -0.5).astype(jnp.bfloat16)) * LOG2E
    masked = float(np.float32(-1e9).astype(jnp.bfloat16)) * LOG2E

    def w_copies(j):
        slot = j % 3
        return [pltpu.make_async_copy(src.bitcast(U32).at[:, j, :], dst.at[slot], wsem.at[slot, i])
                for i, (src, dst) in enumerate(((wk_hbm, wk_v), (wv_hbm, wv_v), (wq_hbm, wq_v)))]

    c_cp = [pltpu.make_async_copy(c_hbm.at[:, pl.ds(t * L, L)], c_v.at[t], sems.at[t]) for t in range(nc)]
    x_cp = pltpu.make_async_copy(x_hbm, x_v, sems.at[nc])
    wo_cp = pltpu.make_async_copy(wo_hbm, wo_v, sems.at[nc + 1])
    ffn_cp = [pltpu.make_async_copy(s, d, sems.at[nc + 2 + i])
              for i, (s, d) in enumerate(((wg_hbm, wg_v), (wu_hbm, wu_v), (wd_hbm, wd_v)))]

    def rows(i):
        return slice(i * BQ, (i + 1) * BQ)

    def proj_kv(slot, hi, k_dst, v_dst):
        w = jnp.concatenate([_half(wk_v[slot], hi), _half(wv_v[slot], hi)], axis=1)
        for i in range(nq):
            kv = _dot(jnp.concatenate([c_v[t, rows(i)] for t in range(nc)], axis=1), w)
            k_dst[rows(i)] = kv[:, :L].astype(BF16)
            v_dst[rows(i)] = kv[:, L:].astype(BF16)

    def proj_q(slot, hi, q_dst):
        w = _half(wq_v[slot], hi)
        for i in range(nq):
            q = _dot(jnp.concatenate([xn_v[t, rows(i)] for t in range(nm)], axis=1), w)
            q_dst[rows(i)] = (q * q_scale).astype(BF16)

    def attend(i, q_ref, k_ref, v_ref):
        r0, ng = i * BQ, BQ // L
        tri = lax.broadcasted_iota(I32, (L, L), 1) <= lax.broadcasted_iota(I32, (L, L), 0)
        s = [[] for _ in range(ng)]
        if i:
            full = _dot_nt(q_ref[rows(i)], k_ref[:r0])
            for g in range(ng):
                s[g] += [full[g * L:(g + 1) * L, t * L:(t + 1) * L] for t in range(r0 // L)]
        for t in range(ng):
            d = _dot_nt(q_ref[r0 + t * L:r0 + BQ], k_ref[r0 + t * L:r0 + (t + 1) * L])
            for g in range(t, ng):
                tile = d[(g - t) * L:(g - t + 1) * L]
                s[g].append(jnp.where(tri, tile, masked) if g == t else tile)
        p, inv = [], []
        for g in range(ng):
            m = s[g][0]
            for tile in s[g][1:]:
                m = jnp.maximum(m, tile)
            m = jnp.max(m, axis=1, keepdims=True)
            e = [jnp.exp2(tile - m) for tile in s[g]]
            tot = e[0]
            for tile in e[1:]:
                tot = tot + tile
            inv.append(1.0 / jnp.sum(tot, axis=1, keepdims=True))
            p.append([tile.astype(BF16) for tile in e])
        nf = r0 // L
        o = [None] * ng
        if i:
            full = _dot(jnp.concatenate([jnp.concatenate(p[g][:nf], axis=1) for g in range(ng)], axis=0),
                        v_ref[:r0])
            o = [full[g * L:(g + 1) * L] for g in range(ng)]
        for t in range(ng):
            d = _dot(jnp.concatenate([p[g][nf + t] for g in range(t, ng)], axis=0),
                     v_ref[r0 + t * L:r0 + (t + 1) * L])
            for g in range(t, ng):
                tile = d[(g - t) * L:(g - t + 1) * L]
                o[g] = tile if o[g] is None else o[g] + tile
        return jnp.concatenate([(o[g] * inv[g]).astype(BF16) for g in range(ng)], axis=0)

    def out_copy(i):
        return pltpu.make_async_copy(x_v.at[rows(i)], out_hbm.at[rows(i)], osem.at[i])

    def pair(j, last):
        for i in range(nq):
            ctx_v[rows(i)] = attend(i, qa, ka, va)
        proj_kv(j % 3, True, kb, vb)
        proj_q(j % 3, True, qb)
        wo = wo_v[pl.ds(pl.multiple_of(j * 2 * L, 2 * L), 2 * L), :]
        for i in (reversed(range(nq)) if last else range(nq)):
            ctx = jnp.concatenate([ctx_v[rows(i)], attend(i, qb, kb, vb)], axis=1)
            y = acc_v[rows(i)] + _dot(ctx, wo)
            if last:
                x_v[rows(i)] = y.astype(BF16)
                out_copy(i).start()
            else:
                acc_v[rows(i)] = y
        if not last:
            proj_kv((j + 1) % 3, False, ka, va)
            proj_q((j + 1) % 3, False, qa)

    def layernorm_and_route():
        wr = wr_ref[...].astype(F32).reshape(1, M)
        lane = lax.broadcasted_iota(I32, (8, L), 1)
        r = [jnp.zeros((8, L), F32) for _ in range(S // (8 * L))]
        for b in range(S // L):
            x = x_v[b * L:(b + 1) * L].astype(F32)
            mean = jnp.sum(x, axis=1, keepdims=True) * (1.0 / M)
            cen = x - mean
            var = _round_bf16(jnp.sum(cen * cen, axis=1, keepdims=True) * (1.0 / M))
            eps = float(np.float32(1e-5).astype(jnp.bfloat16))
            den = _round_bf16(jnp.sqrt(_round_bf16(var + eps)))
            xn = (_round_bf16(x - _round_bf16(mean)) * (1.0 / den)).astype(BF16)
            for t in range(nm):
                xn_v[t, b * L:(b + 1) * L] = xn[:, t * L:(t + 1) * L]
            xf = xn.astype(F32)
            acc_v[b * L:(b + 1) * L] = x + (xf + xf * 0.0)
            score = jnp.sum(xf * wr, axis=1, keepdims=True)
            for g in range(L // 8):
                n = b * (L // 8) + g
                r[n // L] = jnp.where(lane == n % L, score[g * 8:(g + 1) * 8], r[n // L])
        sub = lax.broadcasted_iota(I32, (8, L), 0)
        keys = []
        for a, ra in enumerate(r):
            ra = _round_bf16(ra)
            bits = (pltpu.bitcast(jnp.where(ra == 0.0, 0.0, ra), I32) >> 16) & 0xFFFF
            order = jnp.where(bits >= 0x8000, 0xFFFF - bits, bits + 0x8000)
            order = jnp.where(ra != ra, 0, order)
            tok = (a * L + lane) * 8 + sub
            keys.append(pltpu.bitcast(0x10000000 + order * S + (S - 1 - tok), F32))
        row16 = lax.broadcasted_iota(I32, (16, L), 0)
        xs = [jnp.zeros((8, L), F32) for _ in range(nm)]
        gate = jnp.zeros((8, L), F32)
        for cidx in range(TOPC):
            best = keys[0]
            for kk in keys[1:]:
                best = jnp.maximum(best, kk)
            best = jnp.max(jnp.max(best, axis=0, keepdims=True), axis=1, keepdims=True)
            hit = [kk == best for kk in keys]
            val = jnp.where(hit[0], r[0], 0.0)
            for h, ra in zip(hit[1:], r[1:]):
                val = val + jnp.where(h, ra, 0.0)
            val = jnp.sum(jnp.sum(val, axis=0, keepdims=True), axis=1, keepdims=True)
            gate = jnp.where(sub == cidx, val, gate)
            keys = [jnp.where(h, 0.0, kk) for h, kk in zip(hit, keys)]
            tok = S - 1 - (pltpu.bitcast(best, I32)[0, 0] & (S - 1))
            idx_s[cidx] = tok
            base = pl.multiple_of((tok >> 4) << 4, 16)
            for t in range(nm):
                blk = xn_v[t, pl.ds(base, 16)].astype(F32)
                row = jnp.sum(jnp.where(row16 == (tok & 15), blk, 0.0), axis=0, keepdims=True)
                xs[t] = jnp.where(sub == cidx, row, xs[t])
        xs_v[...] = jnp.concatenate(xs, axis=1)
        gate_v[...] = jax.nn.sigmoid(_round_bf16(gate))

    def routed_ffn():
        for cp in ffn_cp:
            cp.wait()
        xs = xs_v[...].astype(BF16)
        g = _round_bf16(_dot_nt(xs, wg_v[...]))
        u = _round_bf16(_dot_nt(xs, wu_v[...]))
        h = (_round_bf16(g * jax.nn.sigmoid(g)) * u).astype(BF16)
        y = _round_bf16(_dot(h, wd_v[...])) * _round_bf16(gate_v[:, :1])
        for cidx in range(TOPC):
            at = pl.ds(idx_s[cidx], 1)
            acc_v[at, :] = acc_v[at, :] + y[cidx:cidx + 1]

    w0 = w_copies(0)
    for cp in w0[:2] + c_cp + [x_cp, w0[2]] + w_copies(1) + [wo_cp] + ffn_cp:
        cp.start()
    for cp in w0[:2] + c_cp:
        cp.wait()
    proj_kv(0, False, ka, va)
    x_cp.wait()
    w0[2].wait()
    layernorm_and_route()
    proj_q(0, False, qa)
    wo_cp.wait()

    def body(j, carry):
        for cp in w_copies(j + 1):
            cp.wait()

        @pl.when(j + 2 < n_pair)
        def _():
            for cp in w_copies(j + 2):
                cp.start()

        pl.when(j == n_pair // 2)(routed_ffn)
        pair(j, False)
        return carry

    lax.fori_loop(0, n_pair - 1, body, 0)
    pair(n_pair - 1, True)
    for i in range(nq):
        out_copy(i).wait()


@jax.jit
def pallas_parallel_sum__compressed_kv_cla__moe_arch_mod__prompt_kernel(
    A_x: jax.Array,
    A_c_kv: jax.Array,
    A_w_q: jax.Array,
    A_w_uk: jax.Array,
    A_w_uv: jax.Array,
    A_w_o: jax.Array,
    B_x: jax.Array,
    B_w_r: jax.Array,
    B_w_gate: jax.Array,
    B_w_up: jax.Array,
    B_w_down: jax.Array,
):
    del B_x
    _, S, M = A_x.shape
    Dc = A_c_kv.shape[2]
    H = A_w_q.shape[1]
    F = B_w_gate.shape[1]
    hbm = pl.BlockSpec(memory_space=pl.ANY)
    vm = pltpu.VMEM
    head = vm((S, L), BF16)
    out = pl.pallas_call(
        _kernel,
        out_shape=jax.ShapeDtypeStruct((S, M), A_x.dtype),
        in_specs=[hbm] * 6 + [pl.BlockSpec(memory_space=pltpu.VMEM)] + [hbm] * 3,
        out_specs=hbm,
        scratch_shapes=[
            vm((S, M), BF16), vm((Dc // L, S, L), BF16), vm((M // L, S, L), BF16), vm((S, M), F32),
            vm((3, M, L), U32), vm((3, Dc, L), U32), vm((3, Dc, L), U32), vm((H * L, M), BF16),
            vm((F, M), BF16), vm((F, M), BF16), vm((F, M), BF16),
            head, head, head, head, head, head, head,
            vm((TOPC, M), F32), vm((TOPC, L), F32), pltpu.SMEM((TOPC,), I32),
            pltpu.SemaphoreType.DMA((Dc // L + 5,)), pltpu.SemaphoreType.DMA((3, 3)),
            pltpu.SemaphoreType.DMA((S // BQ,)),
        ],
        compiler_params=pltpu.CompilerParams(vmem_limit_bytes=110 * 2**20),
        name="fused_mla_mod",
    )(A_x.reshape(S, M), A_c_kv.reshape(S, Dc), A_w_q, A_w_uk, A_w_uv, A_w_o.reshape(H * L, M),
      B_w_r, B_w_gate.T, B_w_up.T, B_w_down)
    return out.reshape(1, S, M)
```

```python
import math

import jax
import jax.numpy as jnp
import numpy as np
from jax import lax
from jax.experimental import pallas as pl
from jax.experimental.pallas import tpu as pltpu

F32, BF16, U32, I32 = jnp.float32, jnp.bfloat16, jnp.uint32, jnp.int32
L = 128
BQ = 512
CH = 4
LAG = 4
STEP = 32
LAG_LAST = 5
TOPC = 8
FFN_CHUNKS = 12
KEY_BASE = 0x10000000
NT = (((1,), (1,)), ((), ()))
LOG2E = math.log2(math.e)


def _round_bf16(x):
    return x.astype(BF16).astype(F32)


def _dot(a, b):
    return jnp.dot(a, b, preferred_element_type=F32)


def _dot_nt(a, b):
    return lax.dot_general(a, b, NT, preferred_element_type=F32)


def _half(u, hi):
    return pltpu.bitcast((u & np.uint32(0xFFFF0000)) if hi else (u << 16), F32)


def _pack(x):
    if x.shape[0] == 16:
        return pltpu.bitcast(pltpu.pack_elementwise([x[:8], x[8:]], packed_dtype=BF16), U32)
    x = x.reshape(x.shape[0] // 16, 2, 8, L)
    u = pltpu.pack_elementwise([x[:, 0], x[:, 1]], packed_dtype=BF16)
    return pltpu.bitcast(u.reshape(-1, L), U32)


def _rows8(x, hi):
    return jnp.concatenate([x[r:r + 8] for r in range(8 * hi, x.shape[0], 16)], axis=0)


def _origin(i, n):
    return (i & ~15) | ((i & 15) >> n) | ((i << (4 - n)) & 15)


def _unpack(u):
    return pltpu.bitcast(u, BF16)


def _kernel(x_hbm, c_hbm, wq_hbm, wk_hbm, wv_hbm, wo_hbm, wr_ref, wg_hbm, wu_hbm, wd_hbm,
            out_hbm,
            x_v, c_v, xn_v, acc_v, wq_v, wk_v, wv_v, wo_v, wg_v, wu_v, wd_v,
            qa, ka, va, qb, kb, vb, ctx_v, p_v, inv_v, key_v, xs_v, gate_v, idx_s, xsem, csem, fsem, wsem, osem):
    S, M = x_v.shape
    n_pair = wq_hbm.shape[1] // 2
    nm, nc = xn_v.shape[0], c_v.shape[0]
    nq, ng = S // BQ, BQ // L
    q_scale = float(np.float32(L ** -0.5).astype(jnp.bfloat16)) * LOG2E
    masked = float(np.float32(-1e9).astype(jnp.bfloat16)) * LOG2E

    def span(start, size):
        return pl.ds(start if isinstance(start, int) else pl.multiple_of(start, size), size)

    def rows(i):
        return span(i * BQ, BQ)

    def half_rows(lo, hi):
        return slice(lo // 2, hi // 2)

    def prows(i):
        return span(i * (BQ // 2), BQ // 2)

    def w_copies(j):
        slot = j % 3
        srcs = [w.bitcast(U32).at[:, j, :] for w in (wk_hbm, wv_hbm, wq_hbm)]
        srcs.append(wo_hbm.at[span(j * 2 * L, 2 * L)])
        return [pltpu.make_async_copy(src, dst.at[slot], wsem.at[slot, i])
                for i, (src, dst) in enumerate(zip(srcs, (wk_v, wv_v, wq_v, wo_v)))]

    def ffn_copies(j):
        n = wg_v.shape[0] // FFN_CHUNKS
        return [pltpu.make_async_copy(src.at[span(j * n, n)], dst.at[span(j * n, n)], fsem.at[i])
                for i, (src, dst) in enumerate(((wg_hbm, wg_v), (wu_hbm, wu_v), (wd_hbm, wd_v)))]

    def in_copies(i):
        cps = [pltpu.make_async_copy(c_hbm.bitcast(U32).at[prows(i), pl.ds(t * L, L)],
                                     c_v.at[t, prows(i)], csem.at[i, t]) for t in range(nc)]
        return cps + [pltpu.make_async_copy(x_hbm.at[rows(i)], x_v.at[rows(i)], xsem.at[i])]

    def out_copy(i):
        return pltpu.make_async_copy(x_v.at[rows(i)], out_hbm.at[rows(i)], osem.at[i])

    def kv_weights(slot, hi):
        return jnp.concatenate([_half(wk_v[slot], hi), _half(wv_v[slot], hi)], axis=1).astype(BF16)

    def proj_kv(i, w, k_dst, v_dst):
        kv = _dot(jnp.concatenate([_unpack(c_v[t, prows(i)]) for t in range(nc)], axis=1), w)
        k_dst[prows(i)] = _pack(kv[:, :L])
        v_dst[prows(i)] = _pack(kv[:, L:])

        def pace(r):
            at = r * STEP // 16 * 16
            return kv[at % BQ:at % BQ + 16, at // BQ * L:(at // BQ + 1) * L]
        return pace

    def proj_q(i, w, q_dst):
        q = _dot(jnp.concatenate([_unpack(xn_v[t, prows(i)]) for t in range(nm)], axis=1), w)
        q_dst[prows(i)] = _pack(q * q_scale)

    def after(mark, *refs):
        for ref in refs:
            spare = (0,) * (len(ref.shape) - 2) + (slice(S // 2, S // 2 + 8),)
            ref[spare] = pltpu.bitcast(mark, U32)
            pltpu.touch(ref)

    def scores(i, q_ref, k_ref):
        r0 = i * BQ
        tri = _origin(lax.broadcasted_iota(I32, (L, L), 1), 1) <= _origin(lax.broadcasted_iota(I32, (L, L), 0), 2)
        s = [[] for _ in range(ng)]
        if i:
            full = _dot_nt(_unpack(q_ref[prows(i)]), _unpack(k_ref[half_rows(0, r0)]))
            for g in range(ng):
                s[g] += [full[g * L:(g + 1) * L, t * L:(t + 1) * L] for t in range(r0 // L)]
        for t in range(ng):
            lo = r0 + t * L
            d = _dot_nt(_unpack(q_ref[half_rows(lo, r0 + BQ)]), _unpack(k_ref[half_rows(lo, lo + L)]))
            for g in range(t, ng):
                tile = d[(g - t) * L:(g - t + 1) * L]
                s[g].append(jnp.where(tri, tile, masked) if g == t else tile)
        top = []
        for g in range(ng):
            m = s[g][0]
            for tile in s[g][1:]:
                m = jnp.maximum(m, tile)
            top.append(jnp.max(m, axis=1, keepdims=True))
        return s, top, (full[-8:, -L:] if i else s[0][0][:8])

    def softmax(s, top, _, pace, lag):
        go = idx_s[0] >= 0
        invs = []
        for g, m in enumerate(top):
            chunks = [jnp.concatenate(s[g][t:t + CH], axis=1) for t in range(0, len(s[g]), CH)]
            for r in range(0, L, 16):
                tot = None
                mr = jnp.where(go, jnp.broadcast_to(m[r:r + 16], (16, L)), pace((g * L + r) // 16))
                if len(invs) >= lag:
                    mr = jnp.where(go, mr, invs[-lag])
                for n, chunk in enumerate(chunks):
                    e = jnp.exp2(chunk[r:r + 16] - jnp.concatenate([mr] * (chunk.shape[1] // L), axis=1))
                    p_v[half_rows(g * L + r, g * L + r + 16), pl.ds(n * CH * L, e.shape[1])] = _pack(e)
                    for t in range(0, e.shape[1], L):
                        tot = e[:, t:t + L] if tot is None else tot + e[:, t:t + L]
                tot = jnp.sum(tot, axis=1, keepdims=True)
                inv = pl.reciprocal(tot, approx=True)
                inv = inv * (2.0 - tot * inv)
                invs.append(jnp.broadcast_to(inv * (2.0 - tot * inv), (16, L)))
                for hi in (0, 1):
                    inv_v[pl.ds(g * L + r + hi, 8, stride=2)] = invs[-1][8 * hi:8 * hi + 8]

    def context(i, v_ref):
        r0 = i * BQ
        o = [None] * ng
        if i:
            full = _dot(_unpack(p_v[:, :r0]),
                        _unpack(v_ref[half_rows(0, r0)]))
            o = [full[g * L:(g + 1) * L] for g in range(ng)]
        for t in range(ng):
            lo = r0 + t * L
            d = _dot(_unpack(p_v[half_rows(t * L, BQ), lo:lo + L]), _unpack(v_ref[half_rows(lo, lo + L)]))
            for g in range(t, ng):
                tile = d[(g - t) * L:(g - t + 1) * L]
                o[g] = tile if o[g] is None else o[g] + tile
        return _pack(jnp.concatenate(o, axis=0) * inv_v[...])

    def pair(j, last):
        wkv, wq = kv_weights(j % 3, True), _half(wq_v[j % 3], True).astype(BF16)
        for i in range(nq):
            qk = scores(i, qa, ka)
            after(qk[2], c_v, xn_v)
            pace = proj_kv(i, wkv, kb, vb)
            proj_q(i, wq, qb)
            softmax(*qk, pace, LAG_LAST if last else LAG)
            ctx_v[prows(i)] = context(i, va)
        wo = wo_v[j % 3]
        if not last:
            wkv, wq = kv_weights((j + 1) % 3, False), _half(wq_v[(j + 1) % 3], False).astype(BF16)

            def out_proj(i, ctx):
                acc_v[rows(i)] += _dot(jnp.concatenate([_unpack(ctx_v[prows(i)]), ctx], axis=1), wo)

            ctx = None
            for i in range(nq):
                qk = scores(i, qb, kb)
                after(qk[2], c_v, xn_v)
                pace = proj_kv(i, wkv, ka, va)
                proj_q(i, wq, qa)
                softmax(*qk, pace, LAG_LAST if last else LAG)
                if i == nq - 1:
                    out_proj(i - 1, prev)
                ctx = _unpack(context(i, vb))
                if 0 < i < nq - 1:
                    out_proj(i - 1, prev)
                prev = ctx
            out_proj(nq - 1, ctx)
        else:
            def finish(i, ctx):
                y = _dot(ctx, wo[L:])
                x_v[rows(i)] = (acc_v[rows(i)] + y).astype(BF16)
                out_copy(i).start()
                return y

            ctx = None
            for i in reversed(range(nq)):
                qk = scores(i, qb, kb)
                after(qk[2], ctx_v)
                if i < nq - 1:
                    y = finish(i + 1, ctx)
                for b in ((i, i - 1) if i == nq - 1 else () if i == nq - 2 else (i,)):
                    y = _dot(_unpack(ctx_v[prows(b)]), wo[:L])
                    acc_v[rows(b)] += y
                softmax(*qk, lambda r: y[r * 16:r * 16 + 16, :L], LAG_LAST)
                ctx = _unpack(context(i, vb))
            finish(0, ctx)

    lane = lax.broadcasted_iota(I32, (8, L), 1)
    sub = lax.broadcasted_iota(I32, (8, L), 0)

    def layernorm(i):
        wr = wr_ref[...].astype(F32).reshape(1, M)
        eps = float(np.float32(1e-5).astype(jnp.bfloat16))
        r = jnp.zeros((8, L), F32)
        for b in range(ng):
            at = span(i * BQ + b * L, L)
            x = x_v[at].astype(F32)
            mean = jnp.sum(x, axis=1, keepdims=True) * (1.0 / M)
            cen = x - mean
            var = _round_bf16(jnp.sum(cen * cen, axis=1, keepdims=True) * (1.0 / M))
            den = _round_bf16(jnp.sqrt(_round_bf16(var + eps)))
            cen, inv = x - _round_bf16(mean), 1.0 / den
            score = [None, None]
            for t in range(nm):
                cols = slice(t * L, (t + 1) * L)
                u = _pack(cen[:, cols])
                u = pltpu.pack_elementwise([_half(u, hi) * _rows8(inv, hi) for hi in (0, 1)], packed_dtype=BF16)
                u = pltpu.bitcast(u, U32)
                xn_v[t, span((i * BQ + b * L) // 2, L // 2)] = u
                xn = [_half(u, hi) for hi in (0, 1)]
                both = jnp.stack([h.reshape(L // 16, 8, L) for h in xn], axis=1).reshape(L, L)
                acc_v[at, cols] = x[:, cols] + both
                for hi in (0, 1):
                    term = xn[hi] * wr[:, cols]
                    score[hi] = term if t == 0 else score[hi] + term
            score = [jnp.sum(v, axis=1, keepdims=True) for v in score]
            for g in range(L // 8):
                r = jnp.where(lane == b * (L // 8) + g, score[g % 2][g // 2 * 8:g // 2 * 8 + 8], r)
        r = _round_bf16(r)
        bits = (pltpu.bitcast(jnp.where(r == 0.0, 0.0, r), I32) >> 16) & 0xFFFF
        order = jnp.where(r != r, 0, jnp.where(bits >= 0x8000, 0xFFFF - bits, bits + 0x8000))
        key = KEY_BASE + order * S + (S - 1 - (i * BQ + lane * 8 + sub))
        key_v[i] = pltpu.bitcast(jnp.where(lane < BQ // 8, key, 0), F32)

    def route_step(c):
        keys = key_v[...]
        best = jnp.max(jnp.max(jnp.max(keys, axis=0), axis=0, keepdims=True), axis=1, keepdims=True)
        key_v[...] = jnp.where(keys == best, 0.0, keys)
        best = pltpu.bitcast(jnp.broadcast_to(best, (8, L)), I32) - KEY_BASE
        order = best >> (S.bit_length() - 1)
        bits = jnp.where(order >= 0x8000, order - 0x8000, 0xFFFF - order)
        gate_v[...] = jnp.where(sub == c, pltpu.bitcast(bits << 16, F32), gate_v[...])
        tok = S - 1 - (best[0, 0] & (S - 1))
        idx_s[c] = tok
        for t in range(nm):
            u = xn_v[t, pl.ds(((tok >> 4) << 3) | (tok & 7), 1)]
            row = jnp.where((tok & 8) != 0, _half(u, 1), _half(u, 0))
            xs_v[:, t * L:(t + 1) * L] = jnp.where(sub == c, row, xs_v[:, t * L:(t + 1) * L])

    def routed_ffn():
        xs = xs_v[...].astype(BF16)
        g = _round_bf16(_dot_nt(xs, wg_v[...]))
        u = _round_bf16(_dot_nt(xs, wu_v[...]))
        h = (_round_bf16(g * jax.nn.sigmoid(g)) * u).astype(BF16)
        y = _round_bf16(_dot(h, wd_v[...])) * _round_bf16(jax.nn.sigmoid(gate_v[:, :1]))
        for c in range(TOPC):
            at = pl.ds(idx_s[c], 1)
            acc_v[at, :] = acc_v[at, :] + y[c:c + 1]

    w0 = w_copies(0)
    for cp in w0[:3] + in_copies(0) + in_copies(1):
        cp.start()
    xs_v[...] = jnp.zeros(xs_v.shape, F32)
    gate_v[...] = jnp.zeros(gate_v.shape, F32)
    for cp in w0[:3]:
        cp.wait()

    wkv0, wq0 = kv_weights(0, False), _half(wq_v[0], False).astype(BF16)

    def first(i, carry):
        for cp in in_copies(i):
            cp.wait()

        @pl.when(i + 2 < nq)
        def _():
            for cp in in_copies(i + 2):
                cp.start()

        @pl.when(i + 2 == nq)
        def _():
            for cp in [w0[3]] + w_copies(1):
                cp.start()

        proj_kv(i, wkv0, ka, va)
        layernorm(i)
        proj_q(i, wq0, qa)
        return carry

    lax.fori_loop(0, nq, first, 0)
    w0[3].wait()

    def body(j, carry):
        pl.when(j == FFN_CHUNKS + 1)(routed_ffn)
        for cp in w_copies(j + 1):
            cp.wait()

        @pl.when(j + 2 < n_pair)
        def _():
            for cp in w_copies(j + 2):
                cp.start()

        @pl.when(jnp.logical_and(j > 0, j <= FFN_CHUNKS))
        def _():
            for cp in ffn_copies(j - 1):
                cp.wait()

        @pl.when(j < FFN_CHUNKS)
        def _():
            for cp in ffn_copies(j):
                cp.start()

        route_step(j)
        pair(j, False)
        return carry

    lax.fori_loop(0, n_pair - 1, body, 0)
    pair(n_pair - 1, True)
    for i in range(nq):
        out_copy(i).wait()


@jax.jit
def pallas_parallel_sum__compressed_kv_cla__moe_arch_mod__prompt_kernel(
    A_x: jax.Array,
    A_c_kv: jax.Array,
    A_w_q: jax.Array,
    A_w_uk: jax.Array,
    A_w_uv: jax.Array,
    A_w_o: jax.Array,
    B_x: jax.Array,
    B_w_r: jax.Array,
    B_w_gate: jax.Array,
    B_w_up: jax.Array,
    B_w_down: jax.Array,
):
    del B_x
    _, S, M = A_x.shape
    Dc = A_c_kv.shape[2]
    H = A_w_q.shape[1]
    F = B_w_gate.shape[1]
    hbm = pl.BlockSpec(memory_space=pl.ANY)
    vm = pltpu.VMEM
    dma = pltpu.SemaphoreType.DMA
    head = vm((S // 2 + 8, L), U32)
    nq, nc = S // BQ, Dc // L
    out = pl.pallas_call(
        _kernel,
        out_shape=jax.ShapeDtypeStruct((S, M), A_x.dtype),
        in_specs=[hbm] * 6 + [pl.BlockSpec(memory_space=pltpu.VMEM)] + [hbm] * 3,
        out_specs=hbm,
        scratch_shapes=[
            vm((S, M), BF16), vm((nc, S // 2 + 8, L), U32), vm((M // L, S // 2 + 8, L), U32), vm((S, M), F32),
            vm((3, M, L), U32), vm((3, Dc, L), U32), vm((3, Dc, L), U32), vm((3, 2 * L, M), BF16),
            vm((F, M), BF16), vm((F, M), BF16), vm((F, M), BF16),
            head, head, head, head, head, head, head, vm((BQ // 2, S), U32), vm((BQ, L), F32),
            vm((nq, 8, L), F32), vm((TOPC, M), F32), vm((TOPC, L), F32), pltpu.SMEM((H // 2,), I32),
            dma((nq,)), dma((nq, nc)), dma((3,)), dma((3, 4)), dma((nq,)),
        ],
        compiler_params=pltpu.CompilerParams(vmem_limit_bytes=110 * 2**20, disable_bounds_checks=True),
        name="fused_mla_mod",
    )(A_x.reshape(S, M), A_c_kv.reshape(S, Dc), A_w_q, A_w_uk, A_w_uv, A_w_o.reshape(H * L, M),
      B_w_r, B_w_gate.T, B_w_up.T, B_w_down)
    return out.reshape(1, S, M)
```

```python
import math

import jax
import jax.numpy as jnp
import numpy as np
from jax import lax
from jax.experimental import pallas as pl
from jax.experimental.pallas import tpu as pltpu

F32, BF16, U32, I32 = jnp.float32, jnp.bfloat16, jnp.uint32, jnp.int32
L = 128
BQ = 512
CH = 4
LAG = 4
STEP = 32
LAG_LAST = 5
TOPC = 8
FFN_CHUNKS = 12
KEY_BASE = 0x10000000
NT = (((1,), (1,)), ((), ()))
LOG2E = math.log2(math.e)


def _round_bf16(x):
    return x.astype(BF16).astype(F32)


def _dot(a, b):
    return jnp.dot(a, b, preferred_element_type=F32)


def _dot_nt(a, b):
    return lax.dot_general(a, b, NT, preferred_element_type=F32)


def _half(u, hi):
    return pltpu.bitcast((u & np.uint32(0xFFFF0000)) if hi else (u << 16), F32)


def _pack(x):
    if x.shape[0] == 16:
        return pltpu.bitcast(pltpu.pack_elementwise([x[:8], x[8:]], packed_dtype=BF16), U32)
    x = x.reshape(x.shape[0] // 16, 2, 8, L)
    u = pltpu.pack_elementwise([x[:, 0], x[:, 1]], packed_dtype=BF16)
    return pltpu.bitcast(u.reshape(-1, L), U32)


def _widen(u):
    return jnp.stack([_half(u, hi).reshape(-1, 8, L) for hi in (0, 1)], axis=1).reshape(-1, L)


def _origin(i, n):
    return (i & ~15) | ((i & 15) >> n) | ((i << (4 - n)) & 15)


def _unpack(u):
    return pltpu.bitcast(u, BF16)


def _kernel(x_hbm, c_hbm, wq_hbm, wk_hbm, wv_hbm, wo_hbm, wr_ref, wg_hbm, wu_hbm, wd_hbm,
            out_hbm,
            x_v, c_v, xn_v, acc_v, wq_v, wk_v, wv_v, wo_v, wg_v, wu_v, wd_v,
            qa, ka, va, qb, kb, vb, ctx_v, p_v, inv_v, key_v, xs_v, gate_v, idx_s, xsem, csem, fsem, wsem, osem):
    S, M = x_v.shape
    n_pair = wq_hbm.shape[1] // 2
    nm, nc = xn_v.shape[0], c_v.shape[0]
    nq, ng = S // BQ, BQ // L
    q_scale = float(np.float32(L ** -0.5).astype(jnp.bfloat16)) * LOG2E
    masked = float(np.float32(-1e9).astype(jnp.bfloat16)) * LOG2E

    def span(start, size):
        return pl.ds(start if isinstance(start, int) else pl.multiple_of(start, size), size)

    def rows(i):
        return span(i * BQ, BQ)

    def half_rows(lo, hi):
        return slice(lo // 2, hi // 2)

    def prows(i):
        return span(i * (BQ // 2), BQ // 2)

    def w_copies(j):
        slot = j % 3
        srcs = [w.bitcast(U32).at[:, j, :] for w in (wk_hbm, wv_hbm, wq_hbm)]
        srcs.append(wo_hbm.at[span(j * 2 * L, 2 * L)])
        return [pltpu.make_async_copy(src, dst.at[slot], wsem.at[slot, i])
                for i, (src, dst) in enumerate(zip(srcs, (wk_v, wv_v, wq_v, wo_v)))]

    def ffn_copies(j):
        n = wg_v.shape[0] // FFN_CHUNKS
        return [pltpu.make_async_copy(src.at[span(j * n, n)], dst.at[span(j * n, n)], fsem.at[i])
                for i, (src, dst) in enumerate(((wg_hbm, wg_v), (wu_hbm, wu_v), (wd_hbm, wd_v)))]

    def in_copies(i):
        cps = [pltpu.make_async_copy(c_hbm.bitcast(U32).at[prows(i), pl.ds(t * L, L)],
                                     c_v.at[t, prows(i)], csem.at[i, t]) for t in range(nc)]
        return cps + [pltpu.make_async_copy(x_hbm.at[rows(i)], x_v.at[rows(i)], xsem.at[i])]

    def out_copy(i):
        return pltpu.make_async_copy(x_v.at[rows(i)], out_hbm.at[rows(i)], osem.at[i])

    def kv_weights(slot, hi):
        return jnp.concatenate([_half(wk_v[slot], hi), _half(wv_v[slot], hi)], axis=1).astype(BF16)

    def proj_kv(i, w, k_dst, v_dst):
        kv = _dot(jnp.concatenate([_unpack(c_v[t, prows(i)]) for t in range(nc)], axis=1), w)
        k_dst[prows(i)] = _pack(kv[:, :L])
        v_dst[prows(i)] = _pack(kv[:, L:])

        def pace(r):
            at = r * STEP // 16 * 16
            return kv[at % BQ:at % BQ + 16, at // BQ * L:(at // BQ + 1) * L]
        return pace

    def proj_q(i, w, q_dst):
        q = _dot(jnp.concatenate([_unpack(xn_v[t, prows(i)]) for t in range(nm)], axis=1), w)
        q_dst[prows(i)] = _pack(q * q_scale)

    def after(mark, *refs):
        for ref in refs:
            spare = (0,) * (len(ref.shape) - 2) + (slice(S // 2, S // 2 + 8),)
            ref[spare] = pltpu.bitcast(mark, U32)
            pltpu.touch(ref)

    def scores(i, q_ref, k_ref):
        r0 = i * BQ
        tri = _origin(lax.broadcasted_iota(I32, (L, L), 1), 1) <= _origin(lax.broadcasted_iota(I32, (L, L), 0), 2)
        s = [[] for _ in range(ng)]
        if i:
            full = _dot_nt(_unpack(q_ref[prows(i)]), _unpack(k_ref[half_rows(0, r0)]))
            for g in range(ng):
                s[g] += [full[g * L:(g + 1) * L, t * L:(t + 1) * L] for t in range(r0 // L)]
        for t in range(ng):
            lo = r0 + t * L
            d = _dot_nt(_unpack(q_ref[half_rows(lo, r0 + BQ)]), _unpack(k_ref[half_rows(lo, lo + L)]))
            for g in range(t, ng):
                tile = d[(g - t) * L:(g - t + 1) * L]
                s[g].append(jnp.where(tri, tile, masked) if g == t else tile)
        top = []
        for g in range(ng):
            m = s[g][0]
            for tile in s[g][1:]:
                m = jnp.maximum(m, tile)
            top.append(jnp.max(m, axis=1, keepdims=True))
        return s, top, (full[-8:, -L:] if i else s[0][0][:8])

    def softmax(s, top, _, pace, lag):
        go = idx_s[0] >= 0
        invs = []
        for g, m in enumerate(top):
            chunks = [jnp.concatenate(s[g][t:t + CH], axis=1) for t in range(0, len(s[g]), CH)]
            for r in range(0, L, 16):
                tot = None
                mr = jnp.where(go, jnp.broadcast_to(m[r:r + 16], (16, L)), pace((g * L + r) // 16))
                if len(invs) >= lag:
                    mr = jnp.where(go, mr, invs[-lag])
                for n, chunk in enumerate(chunks):
                    e = jnp.exp2(chunk[r:r + 16] - jnp.concatenate([mr] * (chunk.shape[1] // L), axis=1))
                    p_v[half_rows(g * L + r, g * L + r + 16), pl.ds(n * CH * L, e.shape[1])] = _pack(e)
                    for t in range(0, e.shape[1], L):
                        tot = e[:, t:t + L] if tot is None else tot + e[:, t:t + L]
                tot = jnp.sum(tot, axis=1, keepdims=True)
                inv = pl.reciprocal(tot, approx=True)
                inv = inv * (2.0 - tot * inv)
                invs.append(jnp.broadcast_to(inv * (2.0 - tot * inv), (16, L)))
                for hi in (0, 1):
                    inv_v[pl.ds(g * L + r + hi, 8, stride=2)] = invs[-1][8 * hi:8 * hi + 8]

    def context(i, v_ref):
        r0 = i * BQ
        o = [None] * ng
        if i:
            full = _dot(_unpack(p_v[:, :r0]),
                        _unpack(v_ref[half_rows(0, r0)]))
            o = [full[g * L:(g + 1) * L] for g in range(ng)]
        for t in range(ng):
            lo = r0 + t * L
            d = _dot(_unpack(p_v[half_rows(t * L, BQ), lo:lo + L]), _unpack(v_ref[half_rows(lo, lo + L)]))
            for g in range(t, ng):
                tile = d[(g - t) * L:(g - t + 1) * L]
                o[g] = tile if o[g] is None else o[g] + tile
        return _pack(jnp.concatenate(o, axis=0) * inv_v[...])

    def pair(j, last):
        wkv, wq = kv_weights(j % 3, True), _half(wq_v[j % 3], True).astype(BF16)
        for i in range(nq):
            qk = scores(i, qa, ka)
            after(qk[2], c_v, xn_v)
            pace = proj_kv(i, wkv, kb, vb)
            proj_q(i, wq, qb)
            softmax(*qk, pace, LAG_LAST if last else LAG)
            ctx_v[prows(i)] = context(i, va)
        wo = wo_v[j % 3]
        if not last:
            wkv, wq = kv_weights((j + 1) % 3, False), _half(wq_v[(j + 1) % 3], False).astype(BF16)

            def out_proj(i, ctx):
                y = _dot(jnp.concatenate([_unpack(ctx_v[prows(i)]), ctx], axis=1), wo)
                acc_v[rows(i)] = jnp.where(j > 0, acc_v[rows(i)], 0.0) + y

            ctx = None
            for i in range(nq):
                qk = scores(i, qb, kb)
                after(qk[2], c_v, xn_v)
                pace = proj_kv(i, wkv, ka, va)
                proj_q(i, wq, qa)
                softmax(*qk, pace, LAG_LAST if last else LAG)
                if i == nq - 1:
                    out_proj(i - 1, prev)
                ctx = _unpack(context(i, vb))
                if 0 < i < nq - 1:
                    out_proj(i - 1, prev)
                prev = ctx
            out_proj(nq - 1, ctx)
        else:
            def finish(i, ctx):
                y = _dot(ctx, wo[L:])
                x_v[rows(i)] = (acc_v[rows(i)] + y).astype(BF16)
                out_copy(i).start()
                return y

            ctx = None
            for i in reversed(range(nq)):
                qk = scores(i, qb, kb)
                after(qk[2], ctx_v)
                if i < nq - 1:
                    y = finish(i + 1, ctx)
                for b in ((i, i - 1) if i == nq - 1 else () if i == nq - 2 else (i,)):
                    y = _dot(_unpack(ctx_v[prows(b)]), wo[:L])
                    xn = jnp.concatenate([_widen(xn_v[t, prows(b)]) for t in range(nm)], axis=1)
                    acc_v[rows(b)] += y + (x_v[rows(b)].astype(F32) + xn)
                softmax(*qk, lambda r: y[r * 16:r * 16 + 16, :L], LAG_LAST)
                ctx = _unpack(context(i, vb))
            finish(0, ctx)

    lane = lax.broadcasted_iota(I32, (8, L), 1)
    sub = lax.broadcasted_iota(I32, (8, L), 0)

    def layernorm(i):
        eps = float(np.float32(1e-5).astype(jnp.bfloat16))
        for b in range(ng):
            x = x_v[span(i * BQ + b * L, L)].astype(F32)
            mean = jnp.sum(x, axis=1, keepdims=True) * (1.0 / M)
            cen = x - mean
            ssq = jnp.sum(cen * cen, axis=1, keepdims=True)
            both = jnp.zeros((8, L), F32)
            for g in range(L // 8):
                both = jnp.where(lane == g, ssq[8 * g:8 * g + 8], both)
            inv = 1.0 / _round_bf16(jnp.sqrt(_round_bf16(_round_bf16(both * (1.0 / M)) + eps)))
            inv = [jnp.concatenate([jnp.broadcast_to(inv[:, g:g + 1], (8, L)) for g in range(hi, L // 8, 2)], axis=0)
                   for hi in (0, 1)]
            cen = x - _round_bf16(mean)
            for t in range(nm):
                u = _pack(cen[:, t * L:(t + 1) * L])
                u = pltpu.pack_elementwise([_half(u, hi) * inv[hi] for hi in (0, 1)], packed_dtype=BF16)
                xn_v[t, span((i * BQ + b * L) // 2, L // 2)] = pltpu.bitcast(u, U32)

    def rank_keys(i):
        wr = wr_ref[...].astype(F32).reshape(1, M)
        score = []
        for hi in (0, 1):
            v = sum(_half(xn_v[t, prows(i)], hi) * wr[:, t * L:(t + 1) * L] for t in range(nm))
            score.append(jnp.sum(v, axis=1, keepdims=True))
        r = jnp.zeros((8, L), F32)
        for g in range(BQ // 8):
            r = jnp.where(lane == g, score[g % 2][g // 2 * 8:g // 2 * 8 + 8], r)
        r = _round_bf16(r)
        bits = (pltpu.bitcast(jnp.where(r == 0.0, 0.0, r), I32) >> 16) & 0xFFFF
        order = jnp.where(r != r, 0, jnp.where(bits >= 0x8000, 0xFFFF - bits, bits + 0x8000))
        key = KEY_BASE + order * S + (S - 1 - (i * BQ + lane * 8 + sub))
        key_v[i] = pltpu.bitcast(jnp.where(lane < BQ // 8, key, 0), F32)

    def route_step(c):
        keys = key_v[...]
        best = jnp.max(jnp.max(jnp.max(keys, axis=0), axis=0, keepdims=True), axis=1, keepdims=True)
        key_v[...] = jnp.where(keys == best, 0.0, keys)
        best = pltpu.bitcast(jnp.broadcast_to(best, (8, L)), I32) - KEY_BASE
        order = best >> (S.bit_length() - 1)
        bits = jnp.where(order >= 0x8000, order - 0x8000, 0xFFFF - order)
        gate_v[...] = jnp.where(sub == c, pltpu.bitcast(bits << 16, F32), gate_v[...])
        tok = S - 1 - (best[0, 0] & (S - 1))
        idx_s[c] = tok
        for t in range(nm):
            u = xn_v[t, pl.ds(((tok >> 4) << 3) | (tok & 7), 1)]
            row = jnp.where((tok & 8) != 0, _half(u, 1), _half(u, 0))
            xs_v[:, t * L:(t + 1) * L] = jnp.where(sub == c, row, xs_v[:, t * L:(t + 1) * L])

    def routed_ffn():
        xs = xs_v[...].astype(BF16)
        g = _round_bf16(_dot_nt(xs, wg_v[...]))
        u = _round_bf16(_dot_nt(xs, wu_v[...]))
        h = (_round_bf16(g * jax.nn.sigmoid(g)) * u).astype(BF16)
        y = _round_bf16(_dot(h, wd_v[...])) * _round_bf16(jax.nn.sigmoid(gate_v[:, :1]))
        for c in range(TOPC):
            at = pl.ds(idx_s[c], 1)
            acc_v[at, :] = acc_v[at, :] + y[c:c + 1]

    w0 = w_copies(0)
    for cp in w0[:3] + in_copies(0):
        cp.start()
    xs_v[...] = jnp.zeros(xs_v.shape, F32)
    gate_v[...] = jnp.zeros(gate_v.shape, F32)
    w0[0].wait()
    for cp in in_copies(1):
        cp.start()
    for cp in w0[1:3]:
        cp.wait()

    wkv0, wq0 = kv_weights(0, False), _half(wq_v[0], False).astype(BF16)

    def first(i, carry):
        for cp in in_copies(i):
            cp.wait()

        @pl.when(i + 2 < nq)
        def _():
            for cp in in_copies(i + 2):
                cp.start()

        @pl.when(i + 2 == nq)
        def _():
            for cp in [w0[3]] + w_copies(1):
                cp.start()

        proj_kv(i, wkv0, ka, va)
        layernorm(i)
        rank_keys(i)
        proj_q(i, wq0, qa)
        return carry

    lax.fori_loop(0, nq, first, 0)
    w0[3].wait()

    def body(j, carry):
        pl.when(j == FFN_CHUNKS + 1)(routed_ffn)
        for cp in w_copies(j + 1):
            cp.wait()

        @pl.when(j + 2 < n_pair)
        def _():
            for cp in w_copies(j + 2):
                cp.start()

        @pl.when(jnp.logical_and(j > 0, j <= FFN_CHUNKS))
        def _():
            for cp in ffn_copies(j - 1):
                cp.wait()

        @pl.when(j < FFN_CHUNKS)
        def _():
            for cp in ffn_copies(j):
                cp.start()

        route_step(j)
        pair(j, False)
        return carry

    lax.fori_loop(0, n_pair - 1, body, 0)
    pair(n_pair - 1, True)
    for i in range(nq):
        out_copy(i).wait()


@jax.jit
def pallas_parallel_sum__compressed_kv_cla__moe_arch_mod__prompt_kernel(
    A_x: jax.Array,
    A_c_kv: jax.Array,
    A_w_q: jax.Array,
    A_w_uk: jax.Array,
    A_w_uv: jax.Array,
    A_w_o: jax.Array,
    B_x: jax.Array,
    B_w_r: jax.Array,
    B_w_gate: jax.Array,
    B_w_up: jax.Array,
    B_w_down: jax.Array,
):
    del B_x
    _, S, M = A_x.shape
    Dc = A_c_kv.shape[2]
    H = A_w_q.shape[1]
    F = B_w_gate.shape[1]
    hbm = pl.BlockSpec(memory_space=pl.ANY)
    vm = pltpu.VMEM
    dma = pltpu.SemaphoreType.DMA
    head = vm((S // 2 + 8, L), U32)
    nq, nc = S // BQ, Dc // L
    out = pl.pallas_call(
        _kernel,
        out_shape=jax.ShapeDtypeStruct((S, M), A_x.dtype),
        in_specs=[hbm] * 6 + [pl.BlockSpec(memory_space=pltpu.VMEM)] + [hbm] * 3,
        out_specs=hbm,
        scratch_shapes=[
            vm((S, M), BF16), vm((nc, S // 2 + 8, L), U32), vm((M // L, S // 2 + 8, L), U32), vm((S, M), F32),
            vm((3, M, L), U32), vm((3, Dc, L), U32), vm((3, Dc, L), U32), vm((3, 2 * L, M), BF16),
            vm((F, M), BF16), vm((F, M), BF16), vm((F, M), BF16),
            head, head, head, head, head, head, head, vm((BQ // 2, S), U32), vm((BQ, L), F32),
            vm((nq, 8, L), F32), vm((TOPC, M), F32), vm((TOPC, L), F32), pltpu.SMEM((H // 2,), I32),
            dma((nq,)), dma((nq, nc)), dma((3,)), dma((3, 4)), dma((nq,)),
        ],
        compiler_params=pltpu.CompilerParams(vmem_limit_bytes=110 * 2**20, disable_bounds_checks=True),
        name="fused_mla_mod",
    )(A_x.reshape(S, M), A_c_kv.reshape(S, Dc), A_w_q, A_w_uk, A_w_uv, A_w_o.reshape(H * L, M),
      B_w_r, B_w_gate.T, B_w_up.T, B_w_down)
    return out.reshape(1, S, M)
```

```python
import math

import jax
import jax.numpy as jnp
import numpy as np
from jax import lax
from jax.experimental import pallas as pl
from jax.experimental.pallas import tpu as pltpu

F32, BF16, U32, I32 = jnp.float32, jnp.bfloat16, jnp.uint32, jnp.int32
L = 128
BQ = 512
STEP = 16
STEP2 = 16
MARK = 504
STEP_LAST = 16
TOPC = 8
FFN_CHUNKS = 12
KEY_BASE = 0x10000000
NT = (((1,), (1,)), ((), ()))
LOG2E = math.log2(math.e)


def _round_bf16(x):
    return x.astype(BF16).astype(F32)


def _dot(a, b):
    return jnp.dot(a, b, preferred_element_type=F32)


def _dot_nt(a, b):
    return lax.dot_general(a, b, NT, preferred_element_type=F32)


def _half(u, hi):
    return pltpu.bitcast((u & np.uint32(0xFFFF0000)) if hi else (u << 16), F32)


def _pack(x):
    if x.shape[0] == 16:
        return pltpu.bitcast(pltpu.pack_elementwise([x[:8], x[8:]], packed_dtype=BF16), U32)
    x = x.reshape(x.shape[0] // 16, 2, 8, L)
    u = pltpu.pack_elementwise([x[:, 0], x[:, 1]], packed_dtype=BF16)
    return pltpu.bitcast(u.reshape(-1, L), U32)


def _widen(u):
    return jnp.stack([_half(u, hi).reshape(-1, 8, L) for hi in (0, 1)], axis=1).reshape(-1, L)


def _origin(i, n):
    return (i & ~15) | ((i & 15) >> n) | ((i << (4 - n)) & 15)


def _unpack(u):
    return pltpu.bitcast(u, BF16)


def _kernel(x_hbm, c_hbm, wq_hbm, wk_hbm, wv_hbm, wo_hbm, wr_ref, wg_hbm, wu_hbm, wd_hbm,
            out_hbm,
            x_v, c_v, xn_v, acc_v, wq_v, wk_v, wv_v, wo_v, wg_v, wu_v, wd_v,
            q_v, k_v, v_v, p_v, inv_v, key_v, xs_v, gate_v, idx_s, xsem, csem, fsem, wsem, osem):
    S, M = x_v.shape
    F = wg_v.shape[0]
    n_head = wq_hbm.shape[1]
    nm, nc = xn_v.shape[0], c_v.shape[0]
    nq, ng = S // BQ, BQ // L
    q_scale = float(np.float32(L ** -0.5).astype(jnp.bfloat16)) * LOG2E
    masked = float(np.float32(-1e9).astype(jnp.bfloat16)) * LOG2E

    def span(start, size):
        return pl.ds(start if isinstance(start, int) else pl.multiple_of(start, size), size)

    def rows(i):
        return span(i * BQ, BQ)

    def half_rows(lo, hi):
        return slice(lo // 2, hi // 2)

    def prows(i):
        return span(i * (BQ // 2), BQ // 2)

    def w_copies(j):
        slot = j % 3
        srcs = [w.bitcast(U32).at[:, j, :] for w in (wk_hbm, wv_hbm, wq_hbm)]
        srcs.append(wo_hbm.at[span(j * 2 * L, 2 * L)])
        return [pltpu.make_async_copy(src, dst.at[slot], wsem.at[slot, i])
                for i, (src, dst) in enumerate(zip(srcs, (wk_v, wv_v, wq_v, wo_v)))]

    def ffn_copies(lo, n):
        return [pltpu.make_async_copy(src.at[span(lo, n)], dst.at[span(lo, n)], fsem.at[i])
                for i, (src, dst) in enumerate(((wg_hbm, wg_v), (wu_hbm, wu_v), (wd_hbm, wd_v)))]

    def in_copies(i):
        cps = [pltpu.make_async_copy(c_hbm.bitcast(U32).at[prows(i), pl.ds(t * L, L)],
                                     c_v.at[t, prows(i)], csem.at[i, t]) for t in range(nc)]
        return cps + [pltpu.make_async_copy(x_hbm.at[rows(i)], x_v.at[rows(i)], xsem.at[i])]

    def out_copy(i):
        return pltpu.make_async_copy(x_v.at[rows(i)], out_hbm.at[rows(i)], osem.at[i])

    def head_weights(h):
        shift = (16 - 16 * (h % 2)).astype(U32) if not isinstance(h, int) else np.uint32(16 - 16 * (h % 2))
        return [_half(w[h // 2 % 3] << shift, 1).astype(BF16) for w in (wq_v, wk_v, wv_v)]

    def project(i, src, w, dst, scale=None):
        y = _dot(jnp.concatenate([_unpack(src[t, prows(i)]) for t in range(src.shape[0])], axis=1), w)
        dst[prows(i)] = _pack(y if scale is None else y * scale)
        return y

    def after(mark, *refs):
        for ref in refs:
            spare = (0,) * (len(ref.shape) - 2) + (slice(S // 2, S // 2 + 8),)
            ref[spare] = pltpu.bitcast(mark, U32)
            pltpu.touch(ref)

    def scores(i):
        r0 = i * BQ
        tri = _origin(lax.broadcasted_iota(I32, (L, L), 1), 1) <= _origin(lax.broadcasted_iota(I32, (L, L), 0), 2)
        s = [[] for _ in range(ng)]
        if i:
            full = _dot_nt(_unpack(q_v[prows(i)]), _unpack(k_v[half_rows(0, r0)]))
            for g in range(ng):
                s[g] += [full[g * L:(g + 1) * L, t * L:(t + 1) * L] for t in range(r0 // L)]
        for t in range(ng):
            lo = r0 + t * L
            d = _dot_nt(_unpack(q_v[half_rows(lo, r0 + BQ)]), _unpack(k_v[half_rows(lo, lo + L)]))
            for g in range(t, ng):
                tile = d[(g - t) * L:(g - t + 1) * L]
                s[g].append(jnp.where(tri, tile, masked) if g == t else tile)
        top = []
        for g in range(ng):
            m = s[g][0]
            for tile in s[g][1:]:
                m = jnp.maximum(m, tile)
            top.append(jnp.max(m, axis=1, keepdims=True))
        return s, top, (full[MARK:MARK + 8, -L:] if i else s[0][0][:8])

    def context(i, s, top, pace):
        go = idx_s[0] >= 0
        r0 = i * BQ
        tot = [None] * (BQ // 16)
        o = None
        for n in [i] + list(range(i)):
            final = n == max(i - 1, 0)
            for k in range(BQ // 16):
                g, r = divmod(k * 16, L)
                m = jnp.broadcast_to(top[g][r:r + 16], (16, L))
                if pace:
                    m = jnp.where(go, m, jnp.concatenate([pace(k)] * 2, axis=0))
                e = [jnp.exp2(tile[r:r + 16] - m) for tile in s[g][n * ng:(n + 1) * ng]]
                for t, x in enumerate(e):
                    p_v[k * 8:k * 8 + 8, pl.ds(n * BQ + t * L, L)] = _pack(x)
                part = sum(e[1:], e[0])
                tot[k] = part if tot[k] is None else tot[k] + part
                if final:
                    den = jnp.sum(tot[k], axis=1, keepdims=True)
                    inv = pl.reciprocal(den, approx=True)
                    inv = inv * (2.0 - den * inv)
                    tot[k] = jnp.broadcast_to(inv * (2.0 - den * inv), (16, L))
                    for hi in (0, 1):
                        inv_v[pl.ds(k * 16 + hi, 8, stride=2)] = tot[k][8 * hi:8 * hi + 8]
            if n == i:
                part = [None] * ng
                for t in range(ng):
                    lo = r0 + t * L
                    d = _dot(_unpack(p_v[half_rows(t * L, BQ), lo:lo + L]), _unpack(v_v[half_rows(lo, lo + L)]))
                    for g in range(t, ng):
                        tile = d[(g - t) * L:(g - t + 1) * L]
                        part[g] = tile if part[g] is None else part[g] + tile
                part = jnp.concatenate(part, axis=0)
            else:
                part = _dot(_unpack(p_v[:, n * BQ:(n + 1) * BQ]), _unpack(v_v[prows(n)]))
            o = part if o is None else o + part
            pace = follow(part, STEP)
        return _unpack(_pack(o * inv_v[...]))

    def follow(y, step):
        return lambda k: y[k * step // 8 * 8:k * step // 8 * 8 + 8, :L]

    def head(h):
        wq, wk, wv = head_weights(h + 1)
        wo = wo_v[h // 2 % 3, span(h % 2 * L, L)]

        def out_proj(i, ctx):
            acc_v[rows(i)] = jnp.where(h > 0, acc_v[rows(i)], 0.0) + _dot(ctx, wo)

        for i in reversed(range(nq)):
            qk = scores(i)
            after(qk[2], c_v, xn_v)
            k_next = project(i, c_v, wk, k_v)
            project(i, xn_v, wq, q_v, q_scale)
            if i < nq - 1:
                project(i + 1, c_v, wv, v_v)
                out_proj(i + 1, ctx)
            ctx = context(i, *qk[:2], follow(k_next, STEP2))
        out_proj(0, ctx)
        project(0, c_v, wv, v_v)

    def last_head(h):
        wo = wo_v[h // 2 % 3, span(h % 2 * L, L)]

        def finish(i, ctx):
            y = _dot(ctx, wo)
            xn = jnp.concatenate([_widen(xn_v[t, prows(i)]) for t in range(nm)], axis=1)
            x_v[rows(i)] = ((x_v[rows(i)].astype(F32) + xn) + acc_v[rows(i)] + y).astype(BF16)
            out_copy(i).start()
            return follow(y, STEP_LAST)

        for i in reversed(range(nq)):
            qk = scores(i)
            ctx = context(i, *qk[:2], finish(i + 1, ctx) if i < nq - 1 else None)
        finish(0, ctx)

    lane = lax.broadcasted_iota(I32, (8, L), 1)
    sub = lax.broadcasted_iota(I32, (8, L), 0)

    def layernorm(i):
        eps = float(np.float32(1e-5).astype(jnp.bfloat16))
        for b in range(ng):
            x = x_v[span(i * BQ + b * L, L)].astype(F32)
            mean = jnp.sum(x, axis=1, keepdims=True) * (1.0 / M)
            cen = x - mean
            ssq = jnp.sum(cen * cen, axis=1, keepdims=True)
            both = jnp.zeros((8, L), F32)
            for g in range(L // 8):
                both = jnp.where(lane == g, ssq[8 * g:8 * g + 8], both)
            inv = 1.0 / _round_bf16(jnp.sqrt(_round_bf16(_round_bf16(both * (1.0 / M)) + eps)))
            inv = [jnp.concatenate([jnp.broadcast_to(inv[:, g:g + 1], (8, L)) for g in range(hi, L // 8, 2)], axis=0)
                   for hi in (0, 1)]
            cen = x - _round_bf16(mean)
            for t in range(nm):
                u = _pack(cen[:, t * L:(t + 1) * L])
                u = pltpu.pack_elementwise([_half(u, hi) * inv[hi] for hi in (0, 1)], packed_dtype=BF16)
                xn_v[t, span((i * BQ + b * L) // 2, L // 2)] = pltpu.bitcast(u, U32)

    def rank_keys(i):
        wr = wr_ref[...].astype(F32).reshape(1, M)
        score = []
        for hi in (0, 1):
            v = sum(_half(xn_v[t, prows(i)], hi) * wr[:, t * L:(t + 1) * L] for t in range(nm))
            score.append(jnp.sum(v, axis=1, keepdims=True))
        r = jnp.zeros((8, L), F32)
        for g in range(BQ // 8):
            r = jnp.where(lane == g, score[g % 2][g // 2 * 8:g // 2 * 8 + 8], r)
        r = _round_bf16(r)
        bits = (pltpu.bitcast(jnp.where(r == 0.0, 0.0, r), I32) >> 16) & 0xFFFF
        order = jnp.where(r != r, 0, jnp.where(bits >= 0x8000, 0xFFFF - bits, bits + 0x8000))
        key = KEY_BASE + order * S + (S - 1 - (i * BQ + lane * 8 + sub))
        key_v[i] = pltpu.bitcast(jnp.where(lane < BQ // 8, key, 0), F32)

    def route_step(c):
        keys = key_v[...]
        best = jnp.max(jnp.max(jnp.max(keys, axis=0), axis=0, keepdims=True), axis=1, keepdims=True)
        key_v[...] = jnp.where(keys == best, 0.0, keys)
        best = pltpu.bitcast(jnp.broadcast_to(best, (8, L)), I32) - KEY_BASE
        order = best >> (S.bit_length() - 1)
        bits = jnp.where(order >= 0x8000, order - 0x8000, 0xFFFF - order)
        gate_v[...] = jnp.where(sub == c, pltpu.bitcast(bits << 16, F32), gate_v[...])
        tok = S - 1 - (best[0, 0] & (S - 1))
        idx_s[c] = tok
        for t in range(nm):
            u = xn_v[t, pl.ds(((tok >> 4) << 3) | (tok & 7), 1)]
            row = jnp.where((tok & 8) != 0, _half(u, 1), _half(u, 0))
            xs_v[:, t * L:(t + 1) * L] = jnp.where(sub == c, row, xs_v[:, t * L:(t + 1) * L])

    def routed_ffn():
        for cp in ffn_copies(0, F):
            cp.wait()
        xs = xs_v[...].astype(BF16)
        g = _round_bf16(_dot_nt(xs, wg_v[...]))
        u = _round_bf16(_dot_nt(xs, wu_v[...]))
        h = (_round_bf16(g * jax.nn.sigmoid(g)) * u).astype(BF16)
        y = _round_bf16(_dot(h, wd_v[...])) * _round_bf16(jax.nn.sigmoid(gate_v[:, :1]))
        for c in range(TOPC):
            at = pl.ds(idx_s[c], 1)
            acc_v[at, :] = acc_v[at, :] + y[c:c + 1]

    w0 = w_copies(0)
    for cp in w0[:3] + in_copies(0):
        cp.start()
    xs_v[...] = jnp.zeros(xs_v.shape, F32)
    gate_v[...] = jnp.zeros(gate_v.shape, F32)
    w0[0].wait()
    for cp in in_copies(1):
        cp.start()
    for cp in w0[1:3]:
        cp.wait()

    wq0, wk0, wv0 = head_weights(0)

    def first(i, carry):
        for cp in in_copies(i):
            cp.wait()

        @pl.when(i + 2 < nq)
        def _():
            for cp in in_copies(i + 2):
                cp.start()

        @pl.when(i + 2 == nq)
        def _():
            for cp in [w0[3]] + w_copies(1):
                cp.start()

        project(i, c_v, wk0, k_v)
        project(i, c_v, wv0, v_v)
        layernorm(i)
        rank_keys(i)
        project(i, xn_v, wq0, q_v, q_scale)
        return carry

    lax.fori_loop(0, nq, first, 0)
    w0[3].wait()

    def body(h, carry):
        pl.when(h == n_head - 2)(routed_ffn)
        j = h // 2
        even = h % 2 == 0

        @pl.when(jnp.logical_and(even, j + 2 < n_head // 2))
        def _():
            for cp in w_copies(j + 2):
                cp.start()

        @pl.when(jnp.logical_and(~even, j < FFN_CHUNKS))
        def _():
            for cp in ffn_copies(j * (F // FFN_CHUNKS), F // FFN_CHUNKS):
                cp.start()

        route_step(h)
        head(h)

        @pl.when(jnp.logical_and(even, j + 1 < n_head // 2))
        def _():
            for cp in w_copies(j + 1):
                cp.wait()

        return carry

    lax.fori_loop(0, n_head - 1, body, 0)
    last_head(n_head - 1)
    for i in range(nq):
        out_copy(i).wait()


@jax.jit
def pallas_parallel_sum__compressed_kv_cla__moe_arch_mod__prompt_kernel(
    A_x: jax.Array,
    A_c_kv: jax.Array,
    A_w_q: jax.Array,
    A_w_uk: jax.Array,
    A_w_uv: jax.Array,
    A_w_o: jax.Array,
    B_x: jax.Array,
    B_w_r: jax.Array,
    B_w_gate: jax.Array,
    B_w_up: jax.Array,
    B_w_down: jax.Array,
):
    del B_x
    _, S, M = A_x.shape
    Dc = A_c_kv.shape[2]
    H = A_w_q.shape[1]
    F = B_w_gate.shape[1]
    hbm = pl.BlockSpec(memory_space=pl.ANY)
    vm = pltpu.VMEM
    dma = pltpu.SemaphoreType.DMA
    head = vm((S // 2 + 8, L), U32)
    nq, nc = S // BQ, Dc // L
    out = pl.pallas_call(
        _kernel,
        out_shape=jax.ShapeDtypeStruct((S, M), A_x.dtype),
        in_specs=[hbm] * 6 + [pl.BlockSpec(memory_space=pltpu.VMEM)] + [hbm] * 3,
        out_specs=hbm,
        scratch_shapes=[
            vm((S, M), BF16), vm((nc, S // 2 + 8, L), U32), vm((M // L, S // 2 + 8, L), U32), vm((S, M), F32),
            vm((3, M, L), U32), vm((3, Dc, L), U32), vm((3, Dc, L), U32), vm((3, 2 * L, M), BF16),
            vm((F, M), BF16), vm((F, M), BF16), vm((F, M), BF16),
            head, head, head, vm((BQ // 2, S), U32), vm((BQ, L), F32),
            vm((nq, 8, L), F32), vm((TOPC, M), F32), vm((TOPC, L), F32), pltpu.SMEM((H,), I32),
            dma((nq,)), dma((nq, nc)), dma((3,)), dma((3, 4)), dma((nq,)),
        ],
        compiler_params=pltpu.CompilerParams(vmem_limit_bytes=110 * 2**20, disable_bounds_checks=True),
        name="fused_mla_mod",
    )(A_x.reshape(S, M), A_c_kv.reshape(S, Dc), A_w_q, A_w_uk, A_w_uv, A_w_o.reshape(H * L, M),
      B_w_r, B_w_gate.T, B_w_up.T, B_w_down)
    return out.reshape(1, S, M)
```

```python
import functools
import math

import jax
import jax.numpy as jnp
import numpy as np
from jax import lax
from jax.experimental import pallas as pl
from jax.experimental.pallas import tpu as pltpu

F32, BF16, U32, I32 = jnp.float32, jnp.bfloat16, jnp.uint32, jnp.int32
L = 128
BQ = 512
STEP = 16
STEP2 = 16
MARK = 256
STEP_LAST = 16
TOPC = 8
FFN_CHUNKS = 12
KEY_BASE = 0x10000000
NT = (((1,), (1,)), ((), ()))
LOG2E = math.log2(math.e)


def _round_bf16(x):
    return x.astype(BF16).astype(F32)


def _dot(a, b):
    return jnp.dot(a, b, preferred_element_type=F32)


def _dot_nt(a, b):
    return lax.dot_general(a, b, NT, preferred_element_type=F32)


def _half(u, hi):
    return pltpu.bitcast((u & np.uint32(0xFFFF0000)) if hi else (u << 16), F32)


def _pack(x):
    if x.shape[0] == 16:
        return pltpu.bitcast(pltpu.pack_elementwise([x[:8], x[8:]], packed_dtype=BF16), U32)
    x = x.reshape(x.shape[0] // 16, 2, 8, L)
    u = pltpu.pack_elementwise([x[:, 0], x[:, 1]], packed_dtype=BF16)
    return pltpu.bitcast(u.reshape(-1, L), U32)


def _widen(u):
    return jnp.stack([_half(u, hi).reshape(-1, 8, L) for hi in (0, 1)], axis=1).reshape(-1, L)


def _origin(i, n):
    return (i & ~15) | ((i & 15) >> n) | ((i << (4 - n)) & 15)


def _unpack(u):
    return pltpu.bitcast(u, BF16)


def _kernel(x_hbm, c_hbm, wq_hbm, wk_hbm, wv_hbm, wo_hbm, wr_ref, wg_hbm, wu_hbm, wd_hbm,
            out_hbm,
            x_v, c_v, xn_v, acc_v, wq_v, wk_v, wv_v, wo_v, wg_v, wu_v, wd_v,
            q_v, k_v, v_v, p_v, inv_v, low_v, key_v, xs_v, gate_v, idx_s, xsem, csem, fsem, wsem, osem):
    S, M = x_v.shape
    F = wg_v.shape[0]
    n_head = wq_hbm.shape[1]
    nm, nc = xn_v.shape[0], c_v.shape[0]
    nq, ng = S // BQ, BQ // L
    q_scale = float(np.float32(L ** -0.5).astype(jnp.bfloat16)) * LOG2E
    masked = float(np.float32(-1e9).astype(jnp.bfloat16)) * LOG2E

    def span(start, size):
        return pl.ds(start if isinstance(start, int) else pl.multiple_of(start, size), size)

    def rows(i):
        return span(i * BQ, BQ)

    def half_rows(lo, hi):
        return slice(lo // 2, hi // 2)

    def prows(i):
        return span(i * (BQ // 2), BQ // 2)

    def w_copies(j):
        slot = j % 3
        srcs = [w.bitcast(U32).at[:, j, :] for w in (wk_hbm, wv_hbm, wq_hbm)]
        srcs.append(wo_hbm.at[span(j * 2 * L, 2 * L)])
        return [pltpu.make_async_copy(src, dst.at[slot], wsem.at[slot, i])
                for i, (src, dst) in enumerate(zip(srcs, (wk_v, wv_v, wq_v, wo_v)))]

    def ffn_copies(lo, n):
        return [pltpu.make_async_copy(src.at[span(lo, n)], dst.at[span(lo, n)], fsem.at[i])
                for i, (src, dst) in enumerate(((wg_hbm, wg_v), (wu_hbm, wu_v), (wd_hbm, wd_v)))]

    def in_copies(i):
        cps = [pltpu.make_async_copy(c_hbm.bitcast(U32).at[prows(i), pl.ds(t * L, L)],
                                     c_v.at[t, prows(i)], csem.at[i, t]) for t in range(nc)]
        return cps + [x_copy(i)]

    def x_copy(i):
        return pltpu.make_async_copy(x_hbm.at[rows(i)], x_v.at[rows(i)], xsem.at[i])

    def out_copy(i):
        return pltpu.make_async_copy(x_v.at[rows(i)], out_hbm.at[rows(i)], osem.at[i])

    def head_weights(h):
        shift = (16 - 16 * (h % 2)).astype(U32) if not isinstance(h, int) else np.uint32(16 - 16 * (h % 2))
        return [_half(w[h // 2 % 3] << shift, 1).astype(BF16) for w in (wq_v, wk_v, wv_v)]

    def project(i, src, w, dst, scale=None):
        y = _dot(jnp.concatenate([_unpack(src[t, prows(i)]) for t in range(src.shape[0])], axis=1), w)
        dst[prows(i)] = _pack(y if scale is None else y * scale)
        return y

    def after(x, mark):
        return jnp.where(idx_s[0] >= 0, x, jnp.concatenate([mark] * (x.shape[0] // 8), axis=0))

    def hold(ref, mark):
        ref[0, span(S // 2 + 8 * jnp.minimum(idx_s[0], 0), 8)] = pltpu.bitcast(mark, U32)

    def scores(i):
        r0 = i * BQ
        tri = _origin(lax.broadcasted_iota(I32, (L, L), 1), 1) <= _origin(lax.broadcasted_iota(I32, (L, L), 0), 2)
        s = [[] for _ in range(ng)]
        if i:
            full = _dot_nt(_unpack(q_v[prows(i)]), _unpack(k_v[half_rows(0, r0)]))
            for g in range(ng):
                s[g] += [full[g * L:(g + 1) * L, t * L:(t + 1) * L] for t in range(r0 // L)]
        for t in range(ng):
            lo = r0 + t * L
            d = _dot_nt(_unpack(q_v[half_rows(lo, r0 + BQ)]), _unpack(k_v[half_rows(lo, lo + L)]))
            for g in range(t, ng):
                tile = d[(g - t) * L:(g - t + 1) * L]
                s[g].append(jnp.where(tri, tile, masked) if g == t else tile)
        top = []
        for g in range(ng):
            m = s[g][0]
            for tile in s[g][1:]:
                m = jnp.maximum(m, tile)
            top.append(jnp.max(m, axis=1, keepdims=True))
        low = functools.reduce(jnp.minimum, top).reshape(L // 8, 8, 1)
        low_v[...] = jnp.minimum(low_v[...], jnp.min(low, axis=0))
        return s, top, (full[MARK:MARK + 8, -L:] if i else s[0][0][:8])

    def context(i, s, top, pace):
        r0 = i * BQ
        tot = [None] * (BQ // 16)
        for n in [i] + list(range(i)):
            final = n == max(i - 1, 0)
            for k in range(BQ // 16):
                g, r = divmod(k * 16, L)
                m = jnp.broadcast_to(top[g][r:r + 16], (16, L))
                if pace:
                    m = after(m, pace(k))
                e = [jnp.exp2(tile[r:r + 16] - m) for tile in s[g][n * ng:(n + 1) * ng]]
                for t, x in enumerate(e):
                    p_v[k * 8:k * 8 + 8, pl.ds(n * BQ + t * L, L)] = _pack(x)
                part = sum(e[1:], e[0])
                tot[k] = part if n == i else tot[k] + part
                if final:
                    den = jnp.sum(tot[k], axis=1, keepdims=True)
                    inv = pl.reciprocal(den, approx=True)
                    inv = inv * (2.0 - den * inv)
                    inv = jnp.broadcast_to(inv * (2.0 - den * inv), (16, L))
                    for hi in (0, 1):
                        inv_v[pl.ds(k * 16 + hi, 8, stride=2)] = inv[8 * hi:8 * hi + 8]
            if n == i:
                part = [None] * ng
                for t in range(ng):
                    lo = r0 + t * L
                    d = _dot(_unpack(p_v[half_rows(t * L, BQ), lo:lo + L]), _unpack(v_v[half_rows(lo, lo + L)]))
                    for g in range(t, ng):
                        tile = d[(g - t) * L:(g - t + 1) * L]
                        part[g] = tile if part[g] is None else part[g] + tile
                o = part = jnp.concatenate(part, axis=0)
            else:
                part = _dot(_unpack(p_v[:, n * BQ:(n + 1) * BQ]), _unpack(v_v[prows(n)]))
                o = o + part
            pace = follow(part, STEP)
        return _unpack(_pack(o * inv_v[...]))

    def follow(y, step):
        return lambda k: y[k * step // 8 * 8:k * step // 8 * 8 + 8, :L]

    def head(h):
        wq, wk, wv = head_weights(h + 1)
        wo = wo_v[h // 2 % 3, span(h % 2 * L, L)]

        def out_proj(i, ctx):
            acc_v[rows(i)] += _dot(ctx, wo)

        for i in reversed(range(nq)):
            qk = scores(i)
            hold(c_v, qk[2])
            hold(xn_v, qk[2])
            k_next = project(i, c_v, wk, k_v)
            project(i, xn_v, wq, q_v, q_scale)
            if i < nq - 1:
                project(i + 1, c_v, wv, v_v)
                out_proj(i + 1, ctx)
            ctx = context(i, *qk[:2], follow(k_next, STEP2))
        out_proj(0, ctx)
        project(0, c_v, wv, v_v)

    def last_head(h):
        wo = wo_v[h // 2 % 3, span(h % 2 * L, L)]

        def finish(i, ctx):
            y = _dot(ctx, wo)
            result(i * BQ, BQ, y)
            out_copy(i).start()
            return follow(y, STEP_LAST)

        for i in reversed(range(nq)):
            qk = scores(i)
            ctx = context(i, *qk[:2], finish(i + 1, ctx) if i < nq - 1 else None)
        finish(0, ctx)

    lane = lax.broadcasted_iota(I32, (8, L), 1)
    sub = lax.broadcasted_iota(I32, (8, L), 0)

    def layernorm(i):
        eps = float(np.float32(1e-5).astype(jnp.bfloat16))
        for b in range(ng):
            x = x_v[span(i * BQ + b * L, L)].astype(F32)
            mean = jnp.sum(x, axis=1, keepdims=True) * (1.0 / M)
            cen = x - mean
            ssq = jnp.sum(cen * cen, axis=1, keepdims=True)
            both = jnp.zeros((8, L), F32)
            for g in range(L // 8):
                both = jnp.where(lane == g, ssq[8 * g:8 * g + 8], both)
            inv = 1.0 / _round_bf16(jnp.sqrt(_round_bf16(_round_bf16(both * (1.0 / M)) + eps)))
            inv = [jnp.concatenate([jnp.broadcast_to(inv[:, g:g + 1], (8, L)) for g in range(hi, L // 8, 2)], axis=0)
                   for hi in (0, 1)]
            cen = x - _round_bf16(mean)
            for t in range(nm):
                u = _pack(cen[:, t * L:(t + 1) * L])
                u = pltpu.pack_elementwise([_half(u, hi) * inv[hi] for hi in (0, 1)], packed_dtype=BF16)
                xn_v[t, span((i * BQ + b * L) // 2, L // 2)] = pltpu.bitcast(u, U32)

    def rank_keys(i):
        wr = wr_ref[...].astype(F32).reshape(1, M)
        score = []
        for hi in (0, 1):
            v = sum(_half(xn_v[t, prows(i)], hi) * wr[:, t * L:(t + 1) * L] for t in range(nm))
            score.append(jnp.sum(v, axis=1, keepdims=True))
        r = jnp.zeros((8, L), F32)
        for g in range(BQ // 8):
            r = jnp.where(lane == g, score[g % 2][g // 2 * 8:g // 2 * 8 + 8], r)
        r = _round_bf16(r)
        bits = (pltpu.bitcast(jnp.where(r == 0.0, 0.0, r), I32) >> 16) & 0xFFFF
        order = jnp.where(r != r, 0, jnp.where(bits >= 0x8000, 0xFFFF - bits, bits + 0x8000))
        key = KEY_BASE + order * S + (S - 1 - (i * BQ + lane * 8 + sub))
        key_v[i] = pltpu.bitcast(jnp.where(lane < BQ // 8, key, 0), F32)

    def route_step(c):
        keys = key_v[...]
        best = jnp.max(jnp.max(jnp.max(keys, axis=0), axis=0, keepdims=True), axis=1, keepdims=True)
        key_v[...] = jnp.where(keys == best, 0.0, keys)
        best = pltpu.bitcast(jnp.broadcast_to(best, (8, L)), I32) - KEY_BASE
        order = best >> (S.bit_length() - 1)
        bits = jnp.where(order >= 0x8000, order - 0x8000, 0xFFFF - order)
        gate_v[...] = jnp.where(sub == c, pltpu.bitcast(bits << 16, F32), gate_v[...])
        tok = S - 1 - (best[0, 0] & (S - 1))
        idx_s[c] = tok
        for t in range(nm):
            u = xn_v[t, pl.ds(((tok >> 4) << 3) | (tok & 7), 1)]
            row = jnp.where((tok & 8) != 0, _half(u, 1), _half(u, 0))
            xs_v[:, t * L:(t + 1) * L] = jnp.where(sub == c, row, xs_v[:, t * L:(t + 1) * L])

    def routed_ffn():
        for cp in ffn_copies(0, F):
            cp.wait()
        xs = xs_v[...].astype(BF16)
        g = _round_bf16(_dot_nt(xs, wg_v[...]))
        u = _round_bf16(_dot_nt(xs, wu_v[...]))
        h = (_round_bf16(g * jax.nn.sigmoid(g)) * u).astype(BF16)
        y = _round_bf16(_dot(h, wd_v[...])) * _round_bf16(jax.nn.sigmoid(gate_v[:, :1]))
        xs_v[...] = y
        scatter()

    def scatter():
        for c in range(TOPC):
            at = pl.ds(idx_s[c], 1)
            acc_v[at, :] = acc_v[at, :] + xs_v[c:c + 1]

    def clear_acc():
        @pl.loop(0, S // L)
        def _(b):
            acc_v[span(b * L, L)] = jnp.zeros((L, M), F32)

    def result(r0, n, y):
        xn = jnp.concatenate([_widen(xn_v[t, span(r0 // 2, n // 2)]) for t in range(nm)], axis=1)
        at = span(r0, n)
        x_v[at] = ((x_v[at].astype(F32) + xn) + acc_v[at] + y).astype(BF16)

    def redo_unskipped():
        clear_acc()
        scatter()

        @pl.loop(0, n_head)
        def _(h):
            for cp in w_copies(h // 2):
                cp.start()
            for cp in w_copies(h // 2):
                cp.wait()

            @pl.loop(0, nq)
            def _(i):
                wq, wk, wv = head_weights(h)
                project(i, xn_v, wq, q_v, q_scale)
                project(i, c_v, wk, k_v)
                project(i, c_v, wv, v_v)

            @pl.loop(0, S // L)
            def _(b):
                s = _dot_nt(_unpack(q_v[span(b * (L // 2), L // 2)]), _unpack(k_v[...]))
                key = _origin(lax.broadcasted_iota(I32, (L, S), 1), 1)
                query = _origin(lax.broadcasted_iota(I32, (L, S), 0), 2) + b * L
                s = jnp.where(key <= query, s, masked)
                e = jnp.exp2(s - jnp.max(s, axis=1, keepdims=True))
                ctx = _dot((e / jnp.sum(e, axis=1, keepdims=True)).astype(BF16), _unpack(v_v[...]))
                ctx = _unpack(_pack(_unpack(_pack(ctx)).astype(F32)))
                acc_v[span(b * L, L)] += _dot(ctx, wo_v[h // 2 % 3, span(h % 2 * L, L)])

        @pl.loop(0, nq)
        def _(i):
            x_copy(i).start()
            x_copy(i).wait()
            result(i * BQ, BQ, 0.0)
            out_copy(i).start()
            out_copy(i).wait()

    w0 = w_copies(0)
    for cp in w0[:3] + in_copies(0):
        cp.start()
    low_v[...] = jnp.zeros(low_v.shape, F32)
    xs_v[...] = jnp.zeros(xs_v.shape, F32)
    gate_v[...] = jnp.zeros(gate_v.shape, F32)
    clear_acc()
    w0[0].wait()
    for cp in in_copies(1):
        cp.start()
    for cp in w0[1:3]:
        cp.wait()

    wq0, wk0, wv0 = head_weights(0)

    def first(i, carry):
        for cp in in_copies(i):
            cp.wait()

        @pl.when(i + 2 < nq)
        def _():
            for cp in in_copies(i + 2):
                cp.start()

        @pl.when(i + 2 == nq)
        def _():
            for cp in [w0[3]] + w_copies(1):
                cp.start()

        project(i, c_v, wk0, k_v)
        project(i, c_v, wv0, v_v)
        layernorm(i)
        rank_keys(i)
        project(i, xn_v, wq0, q_v, q_scale)
        return carry

    lax.fori_loop(0, nq, first, 0)
    w0[3].wait()

    def body(h, carry):
        pl.when(h == n_head - 2)(routed_ffn)
        j = h // 2
        even = h % 2 == 0

        @pl.when(jnp.logical_and(even, j + 2 < n_head // 2))
        def _():
            for cp in w_copies(j + 2):
                cp.start()

        @pl.when(jnp.logical_and(~even, j < FFN_CHUNKS))
        def _():
            for cp in ffn_copies(j * (F // FFN_CHUNKS), F // FFN_CHUNKS):
                cp.start()

        route_step(h)
        head(h)

        @pl.when(jnp.logical_and(even, j + 1 < n_head // 2))
        def _():
            for cp in w_copies(j + 1):
                cp.wait()

        return carry

    lax.fori_loop(0, n_head - 1, body, 0)
    last_head(n_head - 1)
    sunk = jnp.logical_not(jnp.min(low_v[...]) >= 0.5 * masked)
    for i in range(nq):
        out_copy(i).wait()
    pl.when(sunk)(redo_unskipped)


@jax.jit
def pallas_parallel_sum__compressed_kv_cla__moe_arch_mod__prompt_kernel(
    A_x: jax.Array,
    A_c_kv: jax.Array,
    A_w_q: jax.Array,
    A_w_uk: jax.Array,
    A_w_uv: jax.Array,
    A_w_o: jax.Array,
    B_x: jax.Array,
    B_w_r: jax.Array,
    B_w_gate: jax.Array,
    B_w_up: jax.Array,
    B_w_down: jax.Array,
):
    del B_x
    _, S, M = A_x.shape
    Dc = A_c_kv.shape[2]
    H = A_w_q.shape[1]
    F = B_w_gate.shape[1]
    hbm = pl.BlockSpec(memory_space=pl.ANY)
    vm = pltpu.VMEM
    dma = pltpu.SemaphoreType.DMA
    head = vm((S // 2, L), U32)
    nq, nc = S // BQ, Dc // L
    out = pl.pallas_call(
        _kernel,
        out_shape=jax.ShapeDtypeStruct((S, M), A_x.dtype),
        in_specs=[hbm] * 6 + [pl.BlockSpec(memory_space=pltpu.VMEM)] + [hbm] * 3,
        out_specs=hbm,
        scratch_shapes=[
            vm((S, M), BF16), vm((nc, S // 2 + 8, L), U32), vm((M // L, S // 2 + 8, L), U32), vm((S, M), F32),
            vm((3, M, L), U32), vm((3, Dc, L), U32), vm((3, Dc, L), U32), vm((3, 2 * L, M), BF16),
            vm((F, M), BF16), vm((F, M), BF16), vm((F, M), BF16),
            head, head, head, vm((BQ // 2, S), U32), vm((BQ, L), F32),
            vm((8, L), F32),
            vm((nq, 8, L), F32), vm((TOPC, M), F32), vm((TOPC, L), F32), pltpu.SMEM((H,), I32),
            dma((nq,)), dma((nq, nc)), dma((3,)), dma((3, 4)), dma((nq,)),
        ],
        compiler_params=pltpu.CompilerParams(vmem_limit_bytes=110 * 2**20, disable_bounds_checks=True),
        name="fused_mla_mod",
    )(A_x.reshape(S, M), A_c_kv.reshape(S, Dc), A_w_q, A_w_uk, A_w_uv, A_w_o.reshape(H * L, M),
      B_w_r, B_w_gate.T, B_w_up.T, B_w_down)
    return out.reshape(1, S, M)
```

```python
import functools
import math

import jax
import jax.numpy as jnp
import numpy as np
from jax import lax
from jax.experimental import pallas as pl
from jax.experimental.pallas import tpu as pltpu

F32, BF16, U32, I32 = jnp.float32, jnp.bfloat16, jnp.uint32, jnp.int32
L = 128
BQ = 512
TOPC = 8
FFN_CHUNKS = 12
KEY_BASE = 0x10000000
NT = (((1,), (1,)), ((), ()))
LOG2E = math.log2(math.e)


def _round_bf16(x):
    return x.astype(BF16).astype(F32)


def _dot(a, b):
    return jnp.dot(a, b, preferred_element_type=F32)


def _dot_nt(a, b):
    return lax.dot_general(a, b, NT, preferred_element_type=F32)


def _half(u, hi):
    return pltpu.bitcast((u & np.uint32(0xFFFF0000)) if hi else (u << 16), F32)


def _pack(x):
    if x.shape[0] == 16:
        return pltpu.bitcast(pltpu.pack_elementwise([x[:8], x[8:]], packed_dtype=BF16), U32)
    x = x.reshape(x.shape[0] // 16, 2, 8, L)
    u = pltpu.pack_elementwise([x[:, 0], x[:, 1]], packed_dtype=BF16)
    return pltpu.bitcast(u.reshape(-1, L), U32)


def _widen(u):
    return jnp.stack([_half(u, hi).reshape(-1, 8, L) for hi in (0, 1)], axis=1).reshape(-1, L)


def _origin(i, n):
    return (i & ~15) | ((i & 15) >> n) | ((i << (4 - n)) & 15)


def _unpack(u):
    return pltpu.bitcast(u, BF16)


def _kernel(x_hbm, c_hbm, wq_hbm, wk_hbm, wv_hbm, wo_hbm, wr_ref, wg_hbm, wu_hbm, wd_hbm,
            out_hbm,
            x_v, c_v, xn_v, acc_v, wq_v, wk_v, wv_v, wo_v, wg_v, wu_v, wd_v,
            q_v, k_v, v_v, p_v, inv_v, low_v, key_v, xs_v, gate_v, idx_s, xsem, csem, fsem, wsem, osem):
    S, M = x_v.shape
    F = wg_v.shape[0]
    n_head = wq_hbm.shape[1]
    nm, nc = xn_v.shape[0], c_v.shape[0]
    nq, ng = S // BQ, BQ // L
    q_scale = float(np.float32(L ** -0.5).astype(jnp.bfloat16)) * LOG2E
    masked = float(np.float32(-1e9).astype(jnp.bfloat16)) * LOG2E

    def span(start, size):
        return pl.ds(start if isinstance(start, int) else pl.multiple_of(start, size), size)

    def rows(i):
        return span(i * BQ, BQ)

    def half_rows(lo, hi):
        return slice(lo // 2, hi // 2)

    def prows(i):
        return span(i * (BQ // 2), BQ // 2)

    def w_copies(j):
        slot = j % 3
        srcs = [w.bitcast(U32).at[:, j, :] for w in (wk_hbm, wv_hbm, wq_hbm)]
        srcs.append(wo_hbm.at[span(j * 2 * L, 2 * L)])
        return [pltpu.make_async_copy(src, dst.at[slot], wsem.at[slot, i])
                for i, (src, dst) in enumerate(zip(srcs, (wk_v, wv_v, wq_v, wo_v)))]

    def ffn_copies(lo, n):
        return [pltpu.make_async_copy(src.at[span(lo, n)], dst.at[span(lo, n)], fsem.at[i])
                for i, (src, dst) in enumerate(((wg_hbm, wg_v), (wu_hbm, wu_v), (wd_hbm, wd_v)))]

    def in_copies(i):
        cps = [pltpu.make_async_copy(c_hbm.bitcast(U32).at[prows(i), pl.ds(t * L, L)],
                                     c_v.at[t, prows(i)], csem.at[i, t]) for t in range(nc)]
        return cps + [x_copy(i)]

    def x_copy(i):
        return pltpu.make_async_copy(x_hbm.at[rows(i)], x_v.at[rows(i)], xsem.at[i])

    def out_copy(i):
        return pltpu.make_async_copy(x_v.at[rows(i)], out_hbm.at[rows(i)], osem.at[i])

    def head_weights(h):
        shift = (16 - 16 * (h % 2)).astype(U32) if not isinstance(h, int) else np.uint32(16 - 16 * (h % 2))
        return [_half(w[h // 2 % 3] << shift, 1).astype(BF16) for w in (wq_v, wk_v, wv_v)]

    def project(i, src, w, dst, scale=None):
        y = _dot(jnp.concatenate([_unpack(src[t, prows(i)]) for t in range(src.shape[0])], axis=1), w)
        dst[prows(i)] = _pack(y if scale is None else y * scale)
        return y

    def after(x, mark):
        return jnp.where(idx_s[0] >= 0, x, jnp.concatenate([mark] * (x.shape[0] // 8), axis=0))

    def scores(i):
        r0 = i * BQ
        tri = _origin(lax.broadcasted_iota(I32, (L, L), 1), 1) <= _origin(lax.broadcasted_iota(I32, (L, L), 0), 2)
        s = [[] for _ in range(ng)]
        if i:
            full = _dot_nt(_unpack(q_v[prows(i)]), _unpack(k_v[half_rows(0, r0)]))
            for g in range(ng):
                s[g] += [full[g * L:(g + 1) * L, t * L:(t + 1) * L] for t in range(r0 // L)]
        for t in range(ng):
            lo = r0 + t * L
            d = _dot_nt(_unpack(q_v[half_rows(lo, r0 + BQ)]), _unpack(k_v[half_rows(lo, lo + L)]))
            for g in range(t, ng):
                tile = d[(g - t) * L:(g - t + 1) * L]
                s[g].append(jnp.where(tri, tile, masked) if g == t else tile)
        top = []
        for g in range(ng):
            m = s[g][0]
            for tile in s[g][1:]:
                m = jnp.maximum(m, tile)
            top.append(jnp.max(m, axis=1, keepdims=True))
        low = functools.reduce(jnp.minimum, top).reshape(L // 8, 8, 1)
        low_v[...] = jnp.minimum(low_v[...], jnp.min(low, axis=0))
        return s, top

    def context(i, s, top, pace):
        r0 = i * BQ
        tot = [None] * (BQ // 16)
        for n in [i] + list(range(i)):
            final = n == max(i - 1, 0)
            for k in range(BQ // 16):
                g, r = divmod(k * 16, L)
                m = jnp.broadcast_to(top[g][r:r + 16], (16, L))
                if pace is not None:
                    m = after(m, pace[k * 16:k * 16 + 8, :L])
                e = [jnp.exp2(tile[r:r + 16] - m) for tile in s[g][n * ng:(n + 1) * ng]]
                for t, x in enumerate(e):
                    p_v[k * 8:k * 8 + 8, pl.ds(n * BQ + t * L, L)] = _pack(x)
                part = sum(e[1:], e[0])
                tot[k] = part if n == i else tot[k] + part
                if final:
                    den = jnp.sum(tot[k], axis=1, keepdims=True)
                    inv = pl.reciprocal(den, approx=True)
                    inv = inv * (2.0 - den * inv)
                    inv = jnp.broadcast_to(inv * (2.0 - den * inv), (16, L))
                    for hi in (0, 1):
                        inv_v[pl.ds(k * 16 + hi, 8, stride=2)] = inv[8 * hi:8 * hi + 8]
            if n == i:
                part = [None] * ng
                for t in range(ng):
                    lo = r0 + t * L
                    d = _dot(_unpack(p_v[half_rows(t * L, BQ), lo:lo + L]), _unpack(v_v[half_rows(lo, lo + L)]))
                    for g in range(t, ng):
                        tile = d[(g - t) * L:(g - t + 1) * L]
                        part[g] = tile if part[g] is None else part[g] + tile
                o = part = jnp.concatenate(part, axis=0)
            else:
                part = _dot(_unpack(p_v[:, n * BQ:(n + 1) * BQ]), _unpack(v_v[prows(n)]))
                o = o + part
            pace = part
        return _unpack(_pack(o * inv_v[...]))

    def head(h):
        wq, wk, wv = head_weights(h + 1)
        wo = wo_v[h // 2 % 3, span(h % 2 * L, L)]

        def out_proj(i, ctx):
            acc_v[rows(i)] += _dot(ctx, wo)

        for i in reversed(range(nq)):
            qk = scores(i)
            k_next = project(i, c_v, wk, k_v)
            project(i, xn_v, wq, q_v, q_scale)
            if i < nq - 1:
                out_proj(i + 1, ctx)
                project(i + 1, c_v, wv, v_v)
            ctx = context(i, *qk, k_next)
        out_proj(0, ctx)
        project(0, c_v, wv, v_v)

    def last_head(h):
        wo = wo_v[h // 2 % 3, span(h % 2 * L, L)]

        def finish(i, ctx):
            y = _dot(ctx, wo)
            result(i * BQ, BQ, y)
            out_copy(i).start()
            return y

        for i in reversed(range(nq)):
            qk = scores(i)
            ctx = context(i, *qk, finish(i + 1, ctx) if i < nq - 1 else None)
        finish(0, ctx)

    lane = lax.broadcasted_iota(I32, (8, L), 1)
    sub = lax.broadcasted_iota(I32, (8, L), 0)

    def layernorm(i):
        eps = float(np.float32(1e-5).astype(jnp.bfloat16))
        for b in range(ng):
            x = x_v[span(i * BQ + b * L, L)].astype(F32)
            mean = jnp.sum(x, axis=1, keepdims=True) * (1.0 / M)
            cen = x - mean
            ssq = jnp.sum(cen * cen, axis=1, keepdims=True)
            both = jnp.zeros((8, L), F32)
            for g in range(L // 8):
                both = jnp.where(lane == g, ssq[8 * g:8 * g + 8], both)
            inv = 1.0 / _round_bf16(jnp.sqrt(_round_bf16(_round_bf16(both * (1.0 / M)) + eps)))
            inv = [jnp.concatenate([jnp.broadcast_to(inv[:, g:g + 1], (8, L)) for g in range(hi, L // 8, 2)], axis=0)
                   for hi in (0, 1)]
            cen = x - _round_bf16(mean)
            for t in range(nm):
                u = _pack(cen[:, t * L:(t + 1) * L])
                u = pltpu.pack_elementwise([_half(u, hi) * inv[hi] for hi in (0, 1)], packed_dtype=BF16)
                xn_v[t, span((i * BQ + b * L) // 2, L // 2)] = pltpu.bitcast(u, U32)

    def rank_keys(i):
        wr = wr_ref[...].astype(F32).reshape(1, M)
        score = []
        for hi in (0, 1):
            v = sum(_half(xn_v[t, prows(i)], hi) * wr[:, t * L:(t + 1) * L] for t in range(nm))
            score.append(jnp.sum(v, axis=1, keepdims=True))
        r = jnp.zeros((8, L), F32)
        for g in range(BQ // 8):
            r = jnp.where(lane == g, score[g % 2][g // 2 * 8:g // 2 * 8 + 8], r)
        r = _round_bf16(r)
        bits = (pltpu.bitcast(jnp.where(r == 0.0, 0.0, r), I32) >> 16) & 0xFFFF
        order = jnp.where(r != r, 0, jnp.where(bits >= 0x8000, 0xFFFF - bits, bits + 0x8000))
        key = KEY_BASE + order * S + (S - 1 - (i * BQ + lane * 8 + sub))
        key_v[i] = pltpu.bitcast(jnp.where(lane < BQ // 8, key, 0), F32)

    def route_step(c):
        keys = key_v[...]
        best = jnp.max(jnp.max(jnp.max(keys, axis=0), axis=0, keepdims=True), axis=1, keepdims=True)
        key_v[...] = jnp.where(keys == best, 0.0, keys)
        best = pltpu.bitcast(jnp.broadcast_to(best, (8, L)), I32) - KEY_BASE
        order = best >> (S.bit_length() - 1)
        bits = jnp.where(order >= 0x8000, order - 0x8000, 0xFFFF - order)
        gate_v[...] = jnp.where(sub == c, pltpu.bitcast(bits << 16, F32), gate_v[...])
        tok = S - 1 - (best[0, 0] & (S - 1))
        idx_s[c] = tok
        for t in range(nm):
            u = xn_v[t, pl.ds(((tok >> 4) << 3) | (tok & 7), 1)]
            row = jnp.where((tok & 8) != 0, _half(u, 1), _half(u, 0))
            xs_v[:, t * L:(t + 1) * L] = jnp.where(sub == c, row, xs_v[:, t * L:(t + 1) * L])

    def routed_ffn():
        for cp in ffn_copies(0, F):
            cp.wait()
        xs = xs_v[...].astype(BF16)
        g = _round_bf16(_dot_nt(xs, wg_v[...]))
        u = _round_bf16(_dot_nt(xs, wu_v[...]))
        h = (_round_bf16(g * jax.nn.sigmoid(g)) * u).astype(BF16)
        y = _round_bf16(_dot(h, wd_v[...])) * _round_bf16(jax.nn.sigmoid(gate_v[:, :1]))
        xs_v[...] = y
        scatter()

    def scatter():
        for c in range(TOPC):
            at = pl.ds(idx_s[c], 1)
            acc_v[at, :] = acc_v[at, :] + xs_v[c:c + 1]

    def clear_acc():
        @pl.loop(0, S // L)
        def _(b):
            acc_v[span(b * L, L)] = jnp.zeros((L, M), F32)

    def result(r0, n, y):
        xn = jnp.concatenate([_widen(xn_v[t, span(r0 // 2, n // 2)]) for t in range(nm)], axis=1)
        at = span(r0, n)
        x_v[at] = ((x_v[at].astype(F32) + xn) + acc_v[at] + y).astype(BF16)

    def redo_unskipped():
        clear_acc()
        scatter()

        @pl.loop(0, n_head)
        def _(h):
            for cp in w_copies(h // 2):
                cp.start()
            for cp in w_copies(h // 2):
                cp.wait()

            @pl.loop(0, nq)
            def _(i):
                wq, wk, wv = head_weights(h)
                project(i, xn_v, wq, q_v, q_scale)
                project(i, c_v, wk, k_v)
                project(i, c_v, wv, v_v)

            @pl.loop(0, S // L)
            def _(b):
                s = _dot_nt(_unpack(q_v[span(b * (L // 2), L // 2)]), _unpack(k_v[...]))
                key = _origin(lax.broadcasted_iota(I32, (L, S), 1), 1)
                query = _origin(lax.broadcasted_iota(I32, (L, S), 0), 2) + b * L
                s = jnp.where(key <= query, s, masked)
                e = jnp.exp2(s - jnp.max(s, axis=1, keepdims=True))
                ctx = _dot((e / jnp.sum(e, axis=1, keepdims=True)).astype(BF16), _unpack(v_v[...]))
                ctx = _unpack(_pack(_unpack(_pack(ctx)).astype(F32)))
                acc_v[span(b * L, L)] += _dot(ctx, wo_v[h // 2 % 3, span(h % 2 * L, L)])

        @pl.loop(0, nq)
        def _(i):
            x_copy(i).start()
            x_copy(i).wait()
            result(i * BQ, BQ, 0.0)
            out_copy(i).start()
            out_copy(i).wait()

    w0 = w_copies(0)
    for cp in w0[:3] + in_copies(0):
        cp.start()
    low_v[...] = jnp.zeros(low_v.shape, F32)
    xs_v[...] = jnp.zeros(xs_v.shape, F32)
    gate_v[...] = jnp.zeros(gate_v.shape, F32)
    clear_acc()
    w0[0].wait()
    for cp in in_copies(1):
        cp.start()
    for cp in w0[1:3]:
        cp.wait()

    wq0, wk0, wv0 = head_weights(0)

    def first(i, carry):
        for cp in in_copies(i):
            cp.wait()

        @pl.when(i + 2 < nq)
        def _():
            for cp in in_copies(i + 2):
                cp.start()

        @pl.when(i + 2 == nq)
        def _():
            for cp in [w0[3]] + w_copies(1):
                cp.start()

        project(i, c_v, wk0, k_v)
        project(i, c_v, wv0, v_v)
        layernorm(i)
        rank_keys(i)
        project(i, xn_v, wq0, q_v, q_scale)
        return carry

    lax.fori_loop(0, nq, first, 0)
    w0[3].wait()

    def body(h, carry):
        pl.when(h == n_head - 2)(routed_ffn)
        j = h // 2
        even = h % 2 == 0

        @pl.when(jnp.logical_and(even, j + 2 < n_head // 2))
        def _():
            for cp in w_copies(j + 2):
                cp.start()

        @pl.when(jnp.logical_and(~even, j < FFN_CHUNKS))
        def _():
            for cp in ffn_copies(j * (F // FFN_CHUNKS), F // FFN_CHUNKS):
                cp.start()

        route_step(h)
        head(h)

        @pl.when(jnp.logical_and(even, j + 1 < n_head // 2))
        def _():
            for cp in w_copies(j + 1):
                cp.wait()

        return carry

    lax.fori_loop(0, n_head - 1, body, 0)
    last_head(n_head - 1)
    sunk = jnp.logical_not(jnp.min(low_v[...]) >= 0.5 * masked)
    for i in range(nq):
        out_copy(i).wait()
    pl.when(sunk)(redo_unskipped)


@jax.jit
def pallas_parallel_sum__compressed_kv_cla__moe_arch_mod__prompt_kernel(
    A_x: jax.Array,
    A_c_kv: jax.Array,
    A_w_q: jax.Array,
    A_w_uk: jax.Array,
    A_w_uv: jax.Array,
    A_w_o: jax.Array,
    B_x: jax.Array,
    B_w_r: jax.Array,
    B_w_gate: jax.Array,
    B_w_up: jax.Array,
    B_w_down: jax.Array,
):
    del B_x
    _, S, M = A_x.shape
    Dc = A_c_kv.shape[2]
    H = A_w_q.shape[1]
    F = B_w_gate.shape[1]
    hbm = pl.BlockSpec(memory_space=pl.ANY)
    vm = pltpu.VMEM
    dma = pltpu.SemaphoreType.DMA
    head = vm((S // 2, L), U32)
    nq, nc = S // BQ, Dc // L
    out = pl.pallas_call(
        _kernel,
        out_shape=jax.ShapeDtypeStruct((S, M), A_x.dtype),
        in_specs=[hbm] * 6 + [pl.BlockSpec(memory_space=pltpu.VMEM)] + [hbm] * 3,
        out_specs=hbm,
        scratch_shapes=[
            vm((S, M), BF16), vm((nc, S // 2, L), U32), vm((M // L, S // 2, L), U32), vm((S, M), F32),
            vm((3, M, L), U32), vm((3, Dc, L), U32), vm((3, Dc, L), U32), vm((3, 2 * L, M), BF16),
            vm((F, M), BF16), vm((F, M), BF16), vm((F, M), BF16),
            head, head, head, vm((BQ // 2, S), U32), vm((BQ, L), F32),
            vm((8, L), F32),
            vm((nq, 8, L), F32), vm((TOPC, M), F32), vm((TOPC, L), F32), pltpu.SMEM((H,), I32),
            dma((nq,)), dma((nq, nc)), dma((3,)), dma((3, 4)), dma((nq,)),
        ],
        compiler_params=pltpu.CompilerParams(vmem_limit_bytes=110 * 2**20, disable_bounds_checks=True),
        name="fused_mla_mod",
    )(A_x.reshape(S, M), A_c_kv.reshape(S, Dc), A_w_q, A_w_uk, A_w_uv, A_w_o.reshape(H * L, M),
      B_w_r, B_w_gate.T, B_w_up.T, B_w_down)
    return out.reshape(1, S, M)
```

```python
import functools
import math

import jax
import jax.numpy as jnp
import numpy as np
from jax import lax
from jax.experimental import pallas as pl
from jax.experimental.pallas import tpu as pltpu

F32, BF16, U32, I32 = jnp.float32, jnp.bfloat16, jnp.uint32, jnp.int32
L = 128
BQ = 512
NS = 4
TOPC = 8
FFN_CHUNKS = 12
KEY_BASE = 0x10000000
NT = (((1,), (1,)), ((), ()))
LOG2E = math.log2(math.e)


def _round_bf16(x):
    return x.astype(BF16).astype(F32)


def _dot(a, b):
    return jnp.dot(a, b, preferred_element_type=F32)


def _dot_nt(a, b):
    return lax.dot_general(a, b, NT, preferred_element_type=F32)


def _half(u, hi):
    return pltpu.bitcast((u & np.uint32(0xFFFF0000)) if hi else (u << 16), F32)


def _pack(x):
    if x.shape[0] == 16:
        return pltpu.bitcast(pltpu.pack_elementwise([x[:8], x[8:]], packed_dtype=BF16), U32)
    x = x.reshape(x.shape[0] // 16, 2, 8, L)
    u = pltpu.pack_elementwise([x[:, 0], x[:, 1]], packed_dtype=BF16)
    return pltpu.bitcast(u.reshape(-1, L), U32)


def _widen(u):
    return jnp.stack([_half(u, hi).reshape(-1, 8, L) for hi in (0, 1)], axis=1).reshape(-1, L)


def _origin(i, n):
    return (i & ~15) | ((i & 15) >> n) | ((i << (4 - n)) & 15)


def _unpack(u):
    return pltpu.bitcast(u, BF16)


def _kernel(x_hbm, c_hbm, wq_hbm, wk_hbm, wv_hbm, wo_hbm, wr_ref, wg_hbm, wu_hbm, wd_hbm,
            out_hbm,
            x_v, c_v, xn_v, acc_v, wq_v, wk_v, wv_v, wo_v, wg_v, wu_v, wd_v,
            q_v, k_v, v_v, ctx_v, p_v, inv_v, low_v, key_v, xs_v, gate_v, idx_s, xsem, csem, fsem, wsem, osem):
    S, M = x_v.shape
    F = wg_v.shape[0]
    n_head = wq_hbm.shape[1]
    nm, nc = xn_v.shape[0], c_v.shape[0]
    nq, ng = S // BQ, BQ // L
    q_scale = float(np.float32(L ** -0.5).astype(jnp.bfloat16)) * LOG2E
    masked = float(np.float32(-1e9).astype(jnp.bfloat16)) * LOG2E

    def span(start, size):
        return pl.ds(start if isinstance(start, int) else pl.multiple_of(start, size), size)

    def rows(i):
        return span(i * BQ, BQ)

    def half_rows(lo, hi):
        return slice(lo // 2, hi // 2)

    def prows(i):
        return span(i * (BQ // 2), BQ // 2)

    def w_copies(j):
        slot = j % NS
        srcs = [w.bitcast(U32).at[:, j, :] for w in (wk_hbm, wv_hbm, wq_hbm)]
        srcs.append(wo_hbm.at[span(j * 2 * L, 2 * L)])
        return [pltpu.make_async_copy(src, dst.at[slot], wsem.at[slot, i])
                for i, (src, dst) in enumerate(zip(srcs, (wk_v, wv_v, wq_v, wo_v)))]

    def ffn_copies(lo, n):
        return [pltpu.make_async_copy(src.at[span(lo, n)], dst.at[span(lo, n)], fsem.at[i])
                for i, (src, dst) in enumerate(((wg_hbm, wg_v), (wu_hbm, wu_v), (wd_hbm, wd_v)))]

    def in_copies(i):
        cps = [pltpu.make_async_copy(c_hbm.bitcast(U32).at[prows(i), pl.ds(t * L, L)],
                                     c_v.at[t, prows(i)], csem.at[i, t]) for t in range(nc)]
        return cps + [x_copy(i)]

    def x_copy(i):
        return pltpu.make_async_copy(x_hbm.at[rows(i)], x_v.at[rows(i)], xsem.at[i])

    def out_copy(i):
        return pltpu.make_async_copy(x_v.at[rows(i)], out_hbm.at[rows(i)], osem.at[i])

    def head_weights(h):
        shift = (16 - 16 * (h % 2)).astype(U32) if not isinstance(h, int) else np.uint32(16 - 16 * (h % 2))
        return [_half(w[h // 2 % NS] << shift, 1).astype(BF16) for w in (wq_v, wk_v, wv_v)]

    def project(i, src, w, dst, scale=None):
        y = _dot(jnp.concatenate([_unpack(src[t, prows(i)]) for t in range(src.shape[0])], axis=1), w)
        dst[prows(i)] = _pack(y if scale is None else y * scale)
        return y

    def after(x, mark):
        return jnp.where(idx_s[0] >= 0, x, jnp.concatenate([mark] * (x.shape[0] // 8), axis=0))

    def scores(i):
        r0 = i * BQ
        tri = _origin(lax.broadcasted_iota(I32, (L, L), 1), 1) <= _origin(lax.broadcasted_iota(I32, (L, L), 0), 2)
        s = [[] for _ in range(ng)]
        if i:
            full = _dot_nt(_unpack(q_v[prows(i)]), _unpack(k_v[half_rows(0, r0)]))
            for g in range(ng):
                s[g] += [full[g * L:(g + 1) * L, t * L:(t + 1) * L] for t in range(r0 // L)]
        for t in range(ng):
            lo = r0 + t * L
            d = _dot_nt(_unpack(q_v[half_rows(lo, r0 + BQ)]), _unpack(k_v[half_rows(lo, lo + L)]))
            for g in range(t, ng):
                tile = d[(g - t) * L:(g - t + 1) * L]
                s[g].append(jnp.where(tri, tile, masked) if g == t else tile)
        top = []
        for g in range(ng):
            m = s[g][0]
            for tile in s[g][1:]:
                m = jnp.maximum(m, tile)
            top.append(jnp.max(m, axis=1, keepdims=True))
        low = functools.reduce(jnp.minimum, top).reshape(L // 8, 8, 1)
        low_v[...] = jnp.minimum(low_v[...], jnp.min(low, axis=0))
        return s, top

    def context(i, s, top, pace):
        r0 = i * BQ
        tot = [None] * (BQ // 16)
        for n in [i] + list(range(i)):
            final = n == max(i - 1, 0)
            for k in range(BQ // 16):
                g, r = divmod(k * 16, L)
                m = jnp.broadcast_to(top[g][r:r + 16], (16, L))
                if pace is not None:
                    m = after(m, pace[k * 16:k * 16 + 8, :L])
                e = [jnp.exp2(tile[r:r + 16] - m) for tile in s[g][n * ng:(n + 1) * ng]]
                for t, x in enumerate(e):
                    p_v[k * 8:k * 8 + 8, pl.ds(n * BQ + t * L, L)] = _pack(x)
                part = sum(e[1:], e[0])
                tot[k] = part if n == i else tot[k] + part
                if final:
                    den = jnp.sum(tot[k], axis=1, keepdims=True)
                    inv = pl.reciprocal(den, approx=True)
                    inv = inv * (2.0 - den * inv)
                    inv = jnp.broadcast_to(inv * (2.0 - den * inv), (16, L))
                    for hi in (0, 1):
                        inv_v[pl.ds(k * 16 + hi, 8, stride=2)] = inv[8 * hi:8 * hi + 8]
            if n == i:
                part = [None] * ng
                for t in range(ng):
                    lo = r0 + t * L
                    d = _dot(_unpack(p_v[half_rows(t * L, BQ), lo:lo + L]), _unpack(v_v[half_rows(lo, lo + L)]))
                    for g in range(t, ng):
                        tile = d[(g - t) * L:(g - t + 1) * L]
                        part[g] = tile if part[g] is None else part[g] + tile
                o = part = jnp.concatenate(part, axis=0)
            else:
                part = _dot(_unpack(p_v[:, n * BQ:(n + 1) * BQ]), _unpack(v_v[prows(n)]))
                o = o + part
            pace = part
        return _pack(o * inv_v[...])

    def out_weights(h):
        return wo_v[h // 2 % NS, span(h % 2 * L, L)]

    def left_over(h):
        y = _dot(_unpack(ctx_v[...]), out_weights(max(h - 1, 0) if isinstance(h, int) else jnp.maximum(h - 1, 0)))
        acc_v[rows(0)] += y
        return y

    def head(h):
        wq, wk, wv = head_weights(h + 1)
        wo = out_weights(h)
        for i in reversed(range(nq)):
            qk = scores(i)
            k_next = project(i, c_v, wk, k_v)
            project(i, xn_v, wq, q_v, q_scale)
            if i < nq - 1:
                acc_v[rows(i + 1)] += _dot(_unpack(ctx), wo)
                project(i + 1, c_v, wv, v_v)
            else:
                left_over(h)
            ctx = context(i, *qk, k_next)
        ctx_v[...] = ctx
        project(0, c_v, wv, v_v)

    def last_head(h):
        wo = out_weights(h)

        def finish(i, ctx):
            y = _dot(_unpack(ctx), wo)
            result(i * BQ, BQ, y)
            out_copy(i).start()
            return y

        for i in reversed(range(nq)):
            qk = scores(i)
            ctx = context(i, *qk, finish(i + 1, ctx) if i < nq - 1 else left_over(h))
        finish(0, ctx)

    lane = lax.broadcasted_iota(I32, (8, L), 1)
    sub = lax.broadcasted_iota(I32, (8, L), 0)

    def layernorm(i):
        eps = float(np.float32(1e-5).astype(jnp.bfloat16))
        for b in range(ng):
            x = x_v[span(i * BQ + b * L, L)].astype(F32)
            mean = jnp.sum(x, axis=1, keepdims=True) * (1.0 / M)
            cen = x - mean
            ssq = jnp.sum(cen * cen, axis=1, keepdims=True)
            both = jnp.zeros((8, L), F32)
            for g in range(L // 8):
                both = jnp.where(lane == g, ssq[8 * g:8 * g + 8], both)
            inv = 1.0 / _round_bf16(jnp.sqrt(_round_bf16(_round_bf16(both * (1.0 / M)) + eps)))
            inv = [jnp.concatenate([jnp.broadcast_to(inv[:, g:g + 1], (8, L)) for g in range(hi, L // 8, 2)], axis=0)
                   for hi in (0, 1)]
            cen = x - _round_bf16(mean)
            for t in range(nm):
                u = _pack(cen[:, t * L:(t + 1) * L])
                u = pltpu.pack_elementwise([_half(u, hi) * inv[hi] for hi in (0, 1)], packed_dtype=BF16)
                xn_v[t, span((i * BQ + b * L) // 2, L // 2)] = pltpu.bitcast(u, U32)

    def rank_keys(i):
        wr = wr_ref[...].astype(F32).reshape(1, M)
        score = []
        for hi in (0, 1):
            v = sum(_half(xn_v[t, prows(i)], hi) * wr[:, t * L:(t + 1) * L] for t in range(nm))
            score.append(jnp.sum(v, axis=1, keepdims=True))
        r = jnp.zeros((8, L), F32)
        for g in range(BQ // 8):
            r = jnp.where(lane == g, score[g % 2][g // 2 * 8:g // 2 * 8 + 8], r)
        r = _round_bf16(r)
        bits = (pltpu.bitcast(jnp.where(r == 0.0, 0.0, r), I32) >> 16) & 0xFFFF
        order = jnp.where(r != r, 0, jnp.where(bits >= 0x8000, 0xFFFF - bits, bits + 0x8000))
        key = KEY_BASE + order * S + (S - 1 - (i * BQ + lane * 8 + sub))
        key_v[i] = pltpu.bitcast(jnp.where(lane < BQ // 8, key, 0), F32)

    def route_step(c):
        keys = key_v[...]
        best = jnp.max(jnp.max(jnp.max(keys, axis=0), axis=0, keepdims=True), axis=1, keepdims=True)
        key_v[...] = jnp.where(keys == best, 0.0, keys)
        best = pltpu.bitcast(jnp.broadcast_to(best, (8, L)), I32) - KEY_BASE
        order = best >> (S.bit_length() - 1)
        bits = jnp.where(order >= 0x8000, order - 0x8000, 0xFFFF - order)
        gate_v[...] = jnp.where(sub == c, pltpu.bitcast(bits << 16, F32), gate_v[...])
        tok = S - 1 - (best[0, 0] & (S - 1))
        idx_s[c] = tok
        for t in range(nm):
            u = xn_v[t, pl.ds(((tok >> 4) << 3) | (tok & 7), 1)]
            row = jnp.where((tok & 8) != 0, _half(u, 1), _half(u, 0))
            xs_v[:, t * L:(t + 1) * L] = jnp.where(sub == c, row, xs_v[:, t * L:(t + 1) * L])

    def routed_ffn():
        for cp in ffn_copies(0, F):
            cp.wait()
        xs = xs_v[...].astype(BF16)
        g = _round_bf16(_dot_nt(xs, wg_v[...]))
        u = _round_bf16(_dot_nt(xs, wu_v[...]))
        h = (_round_bf16(g * jax.nn.sigmoid(g)) * u).astype(BF16)
        y = _round_bf16(_dot(h, wd_v[...])) * _round_bf16(jax.nn.sigmoid(gate_v[:, :1]))
        xs_v[...] = y
        scatter()

    def scatter():
        for c in range(TOPC):
            at = pl.ds(idx_s[c], 1)
            acc_v[at, :] = acc_v[at, :] + xs_v[c:c + 1]

    def clear_acc():
        @pl.loop(0, S // L)
        def _(b):
            acc_v[span(b * L, L)] = jnp.zeros((L, M), F32)

    def result(r0, n, y):
        xn = jnp.concatenate([_widen(xn_v[t, span(r0 // 2, n // 2)]) for t in range(nm)], axis=1)
        at = span(r0, n)
        x_v[at] = ((x_v[at].astype(F32) + xn) + acc_v[at] + y).astype(BF16)

    def redo_unskipped():
        clear_acc()
        scatter()

        @pl.loop(0, n_head)
        def _(h):
            for cp in w_copies(h // 2):
                cp.start()
            for cp in w_copies(h // 2):
                cp.wait()

            @pl.loop(0, nq)
            def _(i):
                wq, wk, wv = head_weights(h)
                project(i, xn_v, wq, q_v, q_scale)
                project(i, c_v, wk, k_v)
                project(i, c_v, wv, v_v)

            @pl.loop(0, S // L)
            def _(b):
                s = _dot_nt(_unpack(q_v[span(b * (L // 2), L // 2)]), _unpack(k_v[...]))
                key = _origin(lax.broadcasted_iota(I32, (L, S), 1), 1)
                query = _origin(lax.broadcasted_iota(I32, (L, S), 0), 2) + b * L
                s = jnp.where(key <= query, s, masked)
                e = jnp.exp2(s - jnp.max(s, axis=1, keepdims=True))
                ctx = _dot((e / jnp.sum(e, axis=1, keepdims=True)).astype(BF16), _unpack(v_v[...]))
                ctx = _unpack(_pack(_unpack(_pack(ctx)).astype(F32)))
                acc_v[span(b * L, L)] += _dot(ctx, out_weights(h))

        @pl.loop(0, nq)
        def _(i):
            x_copy(i).start()
            x_copy(i).wait()
            result(i * BQ, BQ, 0.0)
            out_copy(i).start()
            out_copy(i).wait()

    w0 = w_copies(0)
    for cp in w0[:3] + in_copies(0):
        cp.start()
    ctx_v[...] = jnp.zeros(ctx_v.shape, U32)
    low_v[...] = jnp.zeros(low_v.shape, F32)
    xs_v[...] = jnp.zeros(xs_v.shape, F32)
    gate_v[...] = jnp.zeros(gate_v.shape, F32)
    clear_acc()
    w0[0].wait()
    for cp in in_copies(1):
        cp.start()
    for cp in w0[1:3]:
        cp.wait()

    wq0, wk0, wv0 = head_weights(0)

    def first(i, carry):
        for cp in in_copies(i):
            cp.wait()

        @pl.when(i + 2 < nq)
        def _():
            for cp in in_copies(i + 2):
                cp.start()

        @pl.when(i + 2 == nq)
        def _():
            for cp in [w0[3]] + w_copies(1):
                cp.start()

        project(i, c_v, wk0, k_v)
        project(i, c_v, wv0, v_v)
        layernorm(i)
        rank_keys(i)
        project(i, xn_v, wq0, q_v, q_scale)
        return carry

    lax.fori_loop(0, nq, first, 0)
    w0[3].wait()

    def body(h, carry):
        pl.when(h == n_head - 2)(routed_ffn)
        j = h // 2
        even = h % 2 == 0

        @pl.when(jnp.logical_and(even, j + 2 < n_head // 2))
        def _():
            for cp in w_copies(j + 2):
                cp.start()

        @pl.when(jnp.logical_and(~even, j < FFN_CHUNKS))
        def _():
            for cp in ffn_copies(j * (F // FFN_CHUNKS), F // FFN_CHUNKS):
                cp.start()

        route_step(h)
        head(h)

        @pl.when(jnp.logical_and(even, j + 1 < n_head // 2))
        def _():
            for cp in w_copies(j + 1):
                cp.wait()

        return carry

    lax.fori_loop(0, n_head - 1, body, 0)
    last_head(n_head - 1)
    sunk = jnp.logical_not(jnp.min(low_v[...]) >= 0.5 * masked)
    for i in range(nq):
        out_copy(i).wait()
    pl.when(sunk)(redo_unskipped)


@jax.jit
def pallas_parallel_sum__compressed_kv_cla__moe_arch_mod__prompt_kernel(
    A_x: jax.Array,
    A_c_kv: jax.Array,
    A_w_q: jax.Array,
    A_w_uk: jax.Array,
    A_w_uv: jax.Array,
    A_w_o: jax.Array,
    B_x: jax.Array,
    B_w_r: jax.Array,
    B_w_gate: jax.Array,
    B_w_up: jax.Array,
    B_w_down: jax.Array,
):
    del B_x
    _, S, M = A_x.shape
    Dc = A_c_kv.shape[2]
    H = A_w_q.shape[1]
    F = B_w_gate.shape[1]
    hbm = pl.BlockSpec(memory_space=pl.ANY)
    vm = pltpu.VMEM
    dma = pltpu.SemaphoreType.DMA
    head = vm((S // 2, L), U32)
    nq, nc = S // BQ, Dc // L
    out = pl.pallas_call(
        _kernel,
        out_shape=jax.ShapeDtypeStruct((S, M), A_x.dtype),
        in_specs=[hbm] * 6 + [pl.BlockSpec(memory_space=pltpu.VMEM)] + [hbm] * 3,
        out_specs=hbm,
        scratch_shapes=[
            vm((S, M), BF16), vm((nc, S // 2, L), U32), vm((M // L, S // 2, L), U32), vm((S, M), F32),
            vm((NS, M, L), U32), vm((NS, Dc, L), U32), vm((NS, Dc, L), U32), vm((NS, 2 * L, M), BF16),
            vm((F, M), BF16), vm((F, M), BF16), vm((F, M), BF16),
            head, head, head, vm((BQ // 2, L), U32), vm((BQ // 2, S), U32), vm((BQ, L), F32),
            vm((8, L), F32),
            vm((nq, 8, L), F32), vm((TOPC, M), F32), vm((TOPC, L), F32), pltpu.SMEM((H,), I32),
            dma((nq,)), dma((nq, nc)), dma((3,)), dma((NS, 4)), dma((nq,)),
        ],
        compiler_params=pltpu.CompilerParams(vmem_limit_bytes=110 * 2**20, disable_bounds_checks=True),
        name="fused_mla_mod",
    )(A_x.reshape(S, M), A_c_kv.reshape(S, Dc), A_w_q, A_w_uk, A_w_uv, A_w_o.reshape(H * L, M),
      B_w_r, B_w_gate.T, B_w_up.T, B_w_down)
    return out.reshape(1, S, M)
```
